```python
import os as _os
_os.environ.setdefault('JAX_PLATFORMS', 'cpu')
import jax
import jax.numpy as jnp

def _softmax(x, axis=-1):
    return jax.nn.softmax(x, axis=axis)

def _gelu(x):
    return jax.nn.gelu(x, approximate=True)

def _silu(x):
    return jax.nn.silu(x)

def _sigmoid(x):
    return jax.nn.sigmoid(x)

def _layernorm(x, axis=-1, eps=1e-05):
    m = jnp.mean(x, axis=axis, keepdims=True)
    v = jnp.var(x, axis=axis, keepdims=True)
    return (x - m) / jnp.sqrt(v + eps)

def _scatter_add(tgt, idx, src, axis=0):
    return tgt.at[idx].add(src)

def _segment_sum(src, seg, n):
    return jax.ops.segment_sum(src, seg, n)

class _Rng:

    def __init__(self, key):
        self._k = key

    def _next(self):
        self._k, sub = jax.random.split(self._k)
        return sub

    def normal(self, shape):
        return jax.random.normal(self._next(), shape, dtype=jnp.bfloat16)

    def randint(self, lo, hi, shape):
        return jax.random.randint(self._next(), shape, lo, hi, dtype=jnp.int32)

    def uniform(self, shape, lo=0.0, hi=1.0):
        return jax.random.uniform(self._next(), shape, jnp.bfloat16, lo, hi)

    def permutation(self, n):
        return jax.random.permutation(self._next(), n)
kernel_name = 'recurrent_scan__memory_aug_recurrent_mem_tr__mixer_gmlp__prompt'

def setup_inputs():
    _rng = _Rng(jax.random.key(int.from_bytes(__import__("os").urandom(4), "little")))
    _w = lambda a: (lambda t: t.astype(jnp.bfloat16) if jnp.issubdtype(t.dtype, jnp.floating) else t)(jnp.asarray(a))

    def _A_setup():
        B, S, Dm = (1, 2048, 640)
        H, Dh = (32, 128)
        M, seg = (8, 32)
        seg = min(seg, S)
        S = S // seg * seg
        return {'x': _w((lambda *s: _rng.normal(s) * 0.05)(B, S, Dm)), 'mem0': _w((lambda *s: _rng.normal(s) * 0.1)(B, M, Dm)), 'Wq': _w((lambda *s: _rng.normal(s) * 1.6)(Dm, H, Dh) * Dm ** (-0.5)), 'Wk': _w((lambda *s: _rng.normal(s) * 1.6)(Dm, H, Dh) * Dm ** (-0.5)), 'Wv': _w((lambda *s: _rng.normal(s) * 0.1)(Dm, H, Dh) * Dm ** (-0.5)), 'Wo': _w((lambda *s: _rng.normal(s) * 0.1)(H, Dh, Dm) * (H * Dh) ** (-0.5)), 'seg_len': seg}
    _A_in = _A_setup()

    def _B_setup():
        B, S, D, F = (1, 2048, 640, 1728)
        Fh = F // 2
        return {'x': _w((lambda *s: _rng.normal(s) * 0.05)(B, S, D)), 'w_in': _w((lambda *s: _rng.normal(s) * 0.8)(D, 2 * Fh)), 'w_sp': _w(0.01 * (lambda *s: _rng.normal(s) * 0.8)(S, S)), 'b_sp': _w(1.0 + 0.01 * (lambda *s: _rng.normal(s) * 0.05)(S)), 'w_out': _w((lambda *s: _rng.normal(s) * 0.05)(Fh, D))}
    _B_in = _B_setup()
    return {'A_x': _A_in['x'], 'A_mem0': _A_in['mem0'], 'A_Wq': _A_in['Wq'], 'A_Wk': _A_in['Wk'], 'A_Wv': _A_in['Wv'], 'A_Wo': _A_in['Wo'], 'A_seg_len': _A_in['seg_len'], 'B_x': _B_in['x'], 'B_w_in': _B_in['w_in'], 'B_w_sp': _B_in['w_sp'], 'B_b_sp': _B_in['b_sp'], 'B_w_out': _B_in['w_out']}

def reference(A_x, A_mem0, A_Wq, A_Wk, A_Wv, A_Wo, A_seg_len, B_x, B_w_in, B_w_sp, B_b_sp, B_w_out):

    def _A_ref(x, mem0, Wq, Wk, Wv, Wo, seg_len):
        B, S, Dm = x.shape
        H, Dh = (Wq.shape[1], Wq.shape[2])
        M = mem0.shape[1]
        scale = Dh ** (-0.5)
        n_seg = S // seg_len
        L = M + seg_len
        idx = jnp.arange(L)
        mask = (idx[:, None] < M) | (idx[:, None] >= idx[None, :])
        mem = mem0
        outs = []
        for s in range(n_seg):
            xs = x[:, s * seg_len:(s + 1) * seg_len, :].copy()
            h = jnp.concatenate([mem, xs], axis=1)
            q = jnp.einsum('btd,dhe->bhte', h, Wq)
            k = jnp.einsum('btd,dhe->bhte', h, Wk)
            v = jnp.einsum('btd,dhe->bhte', h, Wv)
            scores = jnp.einsum('bhqe,bhke->bhqk', q, k) * scale
            scores = jnp.where(mask[None, None], scores, -1000000000.0)
            p = _softmax(scores, axis=-1)
            o = jnp.einsum('bhqk,bhke->bhqe', p, v)
            o = jnp.einsum('bhte,hed->btd', o, Wo)
            mem = o[:, :M, :].copy()
            outs.append(o[:, M:, :])
        return jnp.concatenate(outs, axis=1)

    def _B_ref(x, w_in, w_sp, b_sp, w_out):
        B, S, D = x.shape
        F = w_in.shape[-1]
        Fh = F // 2
        z = _gelu(jnp.einsum('bsd,df->bsf', x, w_in))
        z1 = z[..., :Fh].copy()
        z2 = _layernorm(z[..., Fh:], axis=-1)
        g = jnp.einsum('ts,bsf->btf', w_sp, z2) + b_sp[None, :, None]
        return jnp.einsum('bsf,fd->bsd', z1 * g, w_out)
    x = A_x
    xn = _layernorm(x, axis=-1)
    s = _A_ref(xn, A_mem0, A_Wq, A_Wk, A_Wv, A_Wo, A_seg_len)
    g = _silu(_B_ref(xn, B_w_in, B_w_sp, B_b_sp, B_w_out))
    return x + s * g
```

```python
import functools

import jax
import jax.numpy as jnp
from jax import lax
from jax.experimental import pallas as pl
from jax.experimental.pallas import tpu as pltpu

F32 = jnp.float32
BF16 = jnp.bfloat16
U32 = jnp.uint32
EPS = 1e-5
NT = (((1,), (1,)), ((), ()))

LANES = 128
KH = 256
MB = 144
LN_ROWS = 32
PACK_ROWS = 40
UNROLL = 4
PEEL = 1
O_GROUPS = (0, 8, 12, 20, 32)
WEIGHTS_NEEDED_AT = 20
FEED_LN, FEED_FINISH, FEED_PACK = 2, 7, 8


def _layernorm(x):
    m = jnp.mean(x, axis=-1, keepdims=True)
    d = x - m
    v = jnp.mean(d * d, axis=-1, keepdims=True)
    return d * lax.rsqrt(v + EPS)


def _gelu2(x):
    c = 0.7978845608028654
    return x + x * jnp.tanh(x * (c + (c * 0.044715) * (x * x)))


def _silu_of_half(y2):
    hy = 0.25 * y2
    return hy + hy * jnp.tanh(hy)


def _recip(l):
    r = pl.reciprocal(l, approx=True)
    return r + r * (1.0 - l * r)


def _pack(w):
    return pltpu.bitcast(w.astype(BF16), U32)


def _unpack(w32):
    return pltpu.bitcast(w32, BF16)


def _dot(a, b):
    return jnp.dot(a, b, preferred_element_type=F32)


def _dot_nt(a, b):
    return lax.dot_general(a, b, NT, preferred_element_type=F32)


def _vreg_sum(x):
    return jnp.sum(x.reshape(x.shape[0] // 8, 8, x.shape[1]), axis=0)


def _after(val, dep):
    return jnp.where(dep * dep < 0.0, pltpu.bitcast(dep, val.dtype), val)


class _SideWork:
    def __init__(self, gens=(), pieces=0, slots=1):
        self.gens, self.rate, self.credit = list(gens), pieces / slots, 0.0
        for g in self.gens:
            next(g)

    def feed(self, m, k=1):
        for t in range(k):
            self.credit += self.rate
            while self.gens and self.credit >= 1.0:
                self.credit -= 1.0
                r = t * (m.shape[0] // 8) // k * 8
                try:
                    self.gens[0].send(m[r:r + 8, :LANES])
                except StopIteration:
                    self.gens.pop(0)

    def drain(self, m):
        while self.gens:
            self.credit += 1.0
            self.feed(m)


def _strassen_left(a):
    return (a[0][0] + a[1][1], a[1][0] + a[1][1], a[0][0], a[1][1],
            a[0][0] + a[0][1], a[1][0] - a[0][0], a[0][1] - a[1][1])


_RIGHT_TERMS = (((0, 0), (1, 1), 1), ((0, 0), None, 0), ((0, 1), (1, 1), -1), ((1, 0), (0, 0), -1),
                ((1, 1), None, 0), ((0, 0), (0, 1), 1), ((1, 0), (1, 1), 1))
_LEFT_SUMS = (0, 1, 4, 5, 6)
_RIGHT_SUMS = (0, 2, 3, 5, 6)


def _strassen_right(p, b):
    first, second, sign = _RIGHT_TERMS[p]
    if second is None:
        return b(*first)
    return b(*first) + b(*second) if sign > 0 else b(*first) - b(*second)


def _strassen_combine(product, add, sub, done=lambda i, n, c: c, plain_left_first=False):
    if plain_left_first:
        m3, m4, m5 = product(2), product(3), product(4)
        c12 = done(0, 1, add(m3, m5))
        m2 = product(1)
        c21 = done(1, 0, add(m2, m4))
    else:
        m2, m4 = product(1), product(3)
        c21 = done(1, 0, add(m2, m4))
        m5, m3 = product(4), product(2)
        c12 = done(0, 1, add(m3, m5))
    d1, d2 = sub(m4, m5), sub(m3, m2)
    m1 = product(0)
    d1, d2 = add(d1, m1), add(d2, m1)
    c11 = done(0, 0, add(d1, product(6)))
    c22 = done(1, 1, add(d2, product(5)))
    return (c11, c12), (c21, c22)


def _segment_ops(heads):
    groups = [("O", a, b) for a, b in zip(O_GROUPS[:-1], O_GROUPS[1:])]
    ops = []
    for t in range(heads):
        ops.append(("P", t))
        if t >= 1:
            ops.append(("S", t - 1))
        if t >= 3:
            ops.append(("V", t - 3))
        if t == groups[0][2] + 3:
            ops.append(groups[0])
    ops += [groups[1], ("S", heads - 1), ("V", heads - 3), groups[2], ("V", heads - 2), ("V", heads - 1)]
    return ops + groups[3:]


def _gating_branch(x_hbm, mem_hbm, wq_hbm, wk_hbm, wv_hbm, wo_hbm, wint_hbm, wsp_hbm, bsp_hbm, wout_hbm,
                   x_v, mem_v, stage_v, wqkv_v, wo_v, wint_v, big_v, bsp_v, wout_v, xn_v, u_v, sem):
    S, D = x_v.shape
    heads, _, DH = wqkv_v.shape[0], wqkv_v.shape[1], wqkv_v.shape[2] // 3
    FH = u_v.shape[1]
    HS, QS = S // 2, S // 4
    HF, QF = FH // 2, FH // 4
    NB = QS // LANES
    n_sem = [0]

    def copy(src, dst):
        n_sem[0] += 1
        return pltpu.make_async_copy(src, dst, sem.at[n_sem[0]])

    def start(cps):
        for cp in cps:
            cp.start()

    def wait(cps):
        for cp in cps:
            cp.wait()

    def x_copies(a, b):
        rs = [slice(q * QS + a * LANES, q * QS + b * LANES) for q in range(4)]
        return [copy(x_hbm.at[r], x_v.at[r]) for r in rs]

    x0_cps, x1_cps, x2_cps = x_copies(0, 1), x_copies(1, 2), x_copies(2, NB)
    w1_cp = copy(wint_hbm.bitcast(U32).at[:HF], wint_v.at[0])
    w2_cp = copy(wint_hbm.bitcast(U32).at[HF:], wint_v.at[1])
    bsp_cp = copy(bsp_hbm, bsp_v)
    wsp_cp = copy(wsp_hbm.bitcast(U32), big_v.at[:HS])
    late_cps = [copy(mem_hbm, mem_v), copy(wout_hbm.bitcast(U32), wout_v), copy(wo_hbm.bitcast(U32), wo_v)]
    qkv_cps = [pltpu.make_async_copy(w.bitcast(U32).at[:, hp, 0], stage_v.at[hp, j], sem.at[0])
               for hp in range(heads // 2) for j, w in enumerate((wq_hbm, wk_hbm, wv_hbm))]

    ZT = HS
    XS = ZT + FH
    WS = XS + HS // 2
    LF = WS + HF

    def tok(q, j, base=0):
        r = base + (q * QS + j * LANES) // 2
        return slice(r, r + LANES // 2)

    def cols(q, j):
        return slice(q * QS + j * LANES, q * QS + (j + 1) * LANES)

    def left_at(p, r0, r1, c0, c1):
        r = LF + (p // 4) * QF
        return slice(r + r0, r + r1), slice((p % 4) * QS + c0, (p % 4) * QS + c1)

    def ln_x(r, n, dep=None):
        xs = []
        for q in (r, HS + r):
            x = x_v[q:q + n, :].astype(F32)
            if dep is not None:
                zero = _after(jnp.zeros((8, LANES), F32), dep)
                x = x + jnp.concatenate([jnp.concatenate([zero] * (n // 8), axis=0)] * (D // LANES), axis=1)
            xs.append(_layernorm(x))
            xn_v[q // 2:(q + n) // 2, :] = _pack(xs[-1])
        for i, p in enumerate(_RIGHT_SUMS):
            t = _strassen_right(p, lambda k, half: xs[half][:, k * KH:(k + 1) * KH])
            big_v[XS + r // 2:XS + (r + n) // 2, i * KH:(i + 1) * KH] = _pack(t)

    def ln_slices(j):
        for q in range(2):
            for r in range(q * QS + j * LANES, q * QS + (j + 1) * LANES, LN_ROWS):
                dep = yield
                ln_x(r, LN_ROWS, dep)

    def w_sums(which):
        left = _strassen_left([[_unpack(wint_v[which, i * HF // 2:(i + 1) * HF // 2, k * KH:(k + 1) * KH])
                                .astype(F32) for k in range(2)] for i in range(2)])
        r = WS + which * (HF // 2)
        for i, p in enumerate(_LEFT_SUMS):
            big_v[r:r + HF // 2, i * KH:(i + 1) * KH] = _pack(left[p])

    def z_block(which, j, f, side, feed):
        def w(i, k):
            r = (i * HF + f) // 2
            return _unpack(wint_v[which, r:r + MB // 2, k * KH:min((k + 1) * KH, D)])

        def x(k, half):
            return _unpack(jnp.concatenate(
                [xn_v[tok(2 * half + q, j), k * KH:min((k + 1) * KH, D)] for q in range(2)], axis=0))

        def left(p):
            if p not in _LEFT_SUMS:
                return w(p - 2, p - 2)
            i, r = _LEFT_SUMS.index(p), WS + (which * HF + f) // 2
            return _unpack(big_v[r:r + MB // 2, i * KH:(i + 1) * KH])

        def right(p):
            if p not in _RIGHT_SUMS:
                return x(p // 4, p // 4)
            i = _RIGHT_SUMS.index(p)
            return _unpack(jnp.concatenate([big_v[tok(q, j, XS), i * KH:(i + 1) * KH] for q in range(2)], axis=0))

        def dot(lhs, rhs):
            m = _dot_nt(lhs, rhs)
            side.feed(m, feed)
            return m

        return _strassen_combine(lambda p: dot(left(p), right(p)), jnp.add, jnp.subtract,
                                 lambda i, half, c: _gelu2(c + dot(w(i, 2), x(2, half))), plain_left_first=True)

    def finish_slices(j, sums, squares):
        ms, rs = [], []
        for half in range(2):
            m = jnp.sum(sums[half], axis=0, keepdims=True) * (1.0 / FH)
            v = jnp.maximum(jnp.sum(squares[half], axis=0, keepdims=True) * (1.0 / FH) - m * m, 0.0)
            r = lax.rsqrt(v + 4.0 * EPS)
            for q in range(2):
                ms.append(jnp.broadcast_to(m[:, q * LANES:(q + 1) * LANES], (8, LANES)))
                rs.append(jnp.broadcast_to(r[:, q * LANES:(q + 1) * LANES], (8, LANES)))
        for f in range(0, QF, 8):
            dep = yield
            mf = [_after(m, dep) for m in ms]
            a = [[(pltpu.bitcast(big_v[ZT + i * QF + f:ZT + i * QF + f + 8, cols(q, j)], F32) - mf[q]) * rs[q]
                  for q in range(4)] for i in range(4)]
            outer = [[_strassen_left([[a[2 * i + i2][2 * k + k2] for k in range(2)] for i in range(2)])
                      for k2 in range(2)] for i2 in range(2)]
            for p in range(7):
                quad = [[outer[i2][k2][p] for k2 in range(2)] for i2 in range(2)]
                if p:
                    dep = yield
                    quad[0][0], quad[1][1] = _after(quad[0][0], dep), _after(quad[1][1], dep)
                for p2, t in enumerate(_strassen_left(quad)):
                    big_v[left_at(7 * p + p2, f, f + 8, j * LANES, (j + 1) * LANES)] = pltpu.bitcast(t, U32)

    def repack_slices():
        low = jnp.full((8, DH), 0xFFFF, U32)
        for hp in range(heads // 2):
            for j in range(3):
                for r in range(0, D // 2, PACK_ROWS):
                    dep = yield
                    m = jnp.concatenate([_after(low, dep)] * (PACK_ROWS // 8), axis=0)
                    even = stage_v[hp, j, pl.ds(2 * r, PACK_ROWS, stride=2), :]
                    odd = stage_v[hp, j, pl.ds(2 * r + 1, PACK_ROWS, stride=2), :]
                    wqkv_v[2 * hp, r:r + PACK_ROWS, j * DH:(j + 1) * DH] = (even & m) | (odd << 16)
                    wqkv_v[2 * hp + 1, r:r + PACK_ROWS, j * DH:(j + 1) * DH] = (even >> 16) | (odd & ~m)

    start(x0_cps + [w2_cp])
    wait(x0_cps)
    for q in range(2):
        ln_x(q * QS, LANES)
    w2_cp.wait()
    start(x1_cps + x2_cps + [bsp_cp, w1_cp, wsp_cp] + qkv_cps + late_cps)
    w_sums(1)

    n_blocks = HF // MB
    products = 11
    ln_pieces = 2 * LANES // LN_ROWS
    finish_pieces = 7 * QF // 8

    side, finishes = _SideWork(), []
    for j in range(NB):
        sums, squares = [0.0, 0.0], [0.0, 0.0]
        for f in range(0, HF, MB):
            slots = 0.9 * (n_blocks - f // MB) * products * FEED_LN
            if (j, f) == (0, MB):
                wait(x1_cps)
            if (j, f) == (1, MB):
                wait(x2_cps)
            if (j, f) in ((0, MB), (1, MB), (2, 0)):
                side = _SideWork([ln_slices(j + 1)], ln_pieces, 0.55 * slots)
            if (j, f) == (NB - 1, 0):
                side = _SideWork([finishes.pop(0)], finish_pieces, slots)
            z = z_block(1, j, f, side, FEED_FINISH if j == NB - 1 else FEED_LN)
            for i in range(2):
                for half in range(2):
                    for q in range(2):
                        big_v[ZT + i * HF + f:ZT + i * HF + f + MB, cols(2 * half + q, j)] = pltpu.bitcast(
                            z[i][half][:, q * LANES:(q + 1) * LANES], U32)
                    partial = _vreg_sum(z[i][half])
                    sums[half] += partial
                    squares[half] += _vreg_sum(z[i][half] * z[i][half])
        side.drain(partial)
        finishes.append(finish_slices(j, sums, squares))
        if j == NB - 2:
            wait([bsp_cp, w1_cp])
            w_sums(0)

    side = _SideWork(finishes, len(finishes) * finish_pieces, 0.9 * NB * n_blocks * products * FEED_FINISH)
    z1 = []
    for j in range(NB):
        z = [z_block(0, j, f, side, FEED_FINISH) for f in range(0, HF, MB)]
        z1.append([jnp.concatenate([blk[i][half] for i in range(2) for blk in z], axis=0) for half in range(2)])
    side.drain(z1[0][0])
    wsp_cp.wait()

    bias = bsp_v[...].astype(F32)
    issued, spatial_side = [0], [_SideWork()]

    def quadrantwise(op):
        return lambda a, b: [[op(a[i][n], b[i][n]) for n in range(2)] for i in range(2)]

    for j in range(NB):
        def outer_product(p):
            if issued[0] == WEIGHTS_NEEDED_AT:
                pltpu.make_async_copy(stage_v, stage_v, sem.at[0]).wait()
                wait(late_cps)
                spatial_side[0] = _SideWork([repack_slices()], (heads // 2) * 3 * (D // 2 // PACK_ROWS),
                                            0.9 * (7 * NB - WEIGHTS_NEEDED_AT) * 7 * FEED_PACK)
            issued[0] += 1
            b = [[_strassen_right(p, lambda k, n: _unpack(
                big_v[tok(2 * n + n2, j), (2 * k + k2) * QS:(2 * k + k2 + 1) * QS]).astype(F32))
                for n2 in range(2)] for k2 in range(2)]

            def inner_product(p2):
                lhs = pltpu.bitcast(big_v[left_at(7 * p + p2, 0, QF, 0, QS)], F32)
                m = _dot_nt(lhs, _strassen_right(p2, lambda k, n: b[k][n]).astype(BF16))
                spatial_side[0].feed(m, FEED_PACK)
                return m

            return _strassen_combine(inner_product, jnp.add, jnp.subtract)

        c = _strassen_combine(outer_product, quadrantwise(jnp.add), quadrantwise(jnp.subtract))
        for half in range(2):
            g = jnp.concatenate(
                [jnp.concatenate([c[i][half][i2][q] for i in range(2) for i2 in range(2)], axis=0)
                 + bias[(2 * half + q) * NB + j:(2 * half + q) * NB + j + 1, :] for q in range(2)], axis=1)
            u = pltpu.bitcast((z1[j][half] * g).astype(BF16).T, U32)
            for q in range(2):
                u_v[tok(2 * half + q, j), :] = u[q * LANES // 2:(q + 1) * LANES // 2]
    spatial_side[0].drain(g)


def _recurrence(out_hbm, x_v, mem_v, wqkv_v, wo_v, wout_v, xn_v, u_v, o_v, out_v, sem_out, seg):
    heads, DH = wqkv_v.shape[0], wqkv_v.shape[2] // 3
    M = mem_v.shape[0]
    n_seg = x_v.shape[0] // seg
    scale = DH ** -0.5
    row = lax.broadcasted_iota(jnp.int32, (M + seg, M + seg), 0)
    col = lax.broadcasted_iota(jnp.int32, (M + seg, M + seg), 1)
    ops = _segment_ops(heads)

    def rows(s, n):
        return pl.ds(s * n, n) if isinstance(s, int) else pl.ds(pl.multiple_of(s * n, n), n)

    def segment(s, mem, last=False):
        q0 = M if last else 0
        mask = ((row < M) | (row >= col))[q0:]
        h = jnp.concatenate([mem, _unpack(xn_v[rows(s, seg // 2), :]).astype(F32)], axis=0)
        q, kv, probs, acc = {}, {}, {}, None
        for op, a, *rest in ops:
            if op == "P":
                if last:
                    q[a] = _dot(h[q0:], _unpack(wqkv_v[a, :, :DH]))
                    kv[a] = _dot(h, _unpack(wqkv_v[a, :, DH:]))
                else:
                    qkv = _dot(h, _unpack(wqkv_v[a]))
                    q[a], kv[a] = qkv[:, :DH], qkv[:, DH:]
            elif op == "S":
                scores = jnp.where(mask, _dot_nt(q.pop(a), kv[a][:, :DH]) * scale, -1e9)
                e = jnp.exp(scores - jnp.max(scores, axis=-1, keepdims=True))
                probs[a] = e, _recip(jnp.sum(e, axis=-1, keepdims=True))
            elif op == "V":
                e, inv = probs.pop(a)
                o_v[q0:, a * DH:(a + 1) * DH] = _dot(e, kv.pop(a)[:, DH:]) * inv
            else:
                b = rest[0]
                part = _dot(o_v[q0:, a * DH:b * DH], _unpack(wo_v[a * DH // 2:b * DH // 2, :]))
                acc = part if acc is None else acc + part
        gate = _silu_of_half(_dot(_unpack(u_v[rows(s, seg // 2), :]), _unpack(wout_v[...])))
        r = rows(s, seg)
        out_v[r, :] = (x_v[r, :].astype(F32) + acc[M - q0:, :] * gate).astype(out_v.dtype)
        pltpu.make_async_copy(out_v.at[r], out_hbm.at[r], sem_out).start()
        return acc[:M, :]

    def body(i, mem):
        for k in range(UNROLL):
            mem = segment(PEEL + i * UNROLL + k, mem)
        return mem

    n_loop = n_seg // UNROLL - 1
    mem = mem_v[...].astype(F32)
    for s in range(PEEL):
        mem = segment(s, mem)
    mem = lax.fori_loop(0, n_loop, body, mem)
    for s in range(PEEL + n_loop * UNROLL, n_seg):
        mem = segment(s, mem, last=s == n_seg - 1)
    pltpu.make_async_copy(out_v, out_hbm, sem_out).wait()


def _kernel(x_hbm, mem_hbm, wq_hbm, wk_hbm, wv_hbm, wo_hbm, wint_hbm, wsp_hbm, bsp_hbm, wout_hbm, out_hbm,
            x_v, mem_v, stage_v, wqkv_v, wo_v, wint_v, big_v, bsp_v, wout_v, xn_v, u_v, o_v, out_v,
            sem, sem_out, *, seg):
    _gating_branch(x_hbm, mem_hbm, wq_hbm, wk_hbm, wv_hbm, wo_hbm, wint_hbm, wsp_hbm, bsp_hbm, wout_hbm,
                   x_v, mem_v, stage_v, wqkv_v, wo_v, wint_v, big_v, bsp_v, wout_v, xn_v, u_v, sem)
    _recurrence(out_hbm, x_v, mem_v, wqkv_v, wo_v, wout_v, xn_v, u_v, o_v, out_v, sem_out, seg)


@functools.partial(jax.jit, static_argnames=("A_seg_len",))
def pallas_recurrent_scan__memory_aug_recurrent_mem_tr__mixer_gmlp__prompt_kernel(
    A_x, A_mem0, A_Wq, A_Wk, A_Wv, A_Wo, A_seg_len, B_x, B_w_in, B_w_sp, B_b_sp, B_w_out,
):
    del B_x
    B, S, D = A_x.shape
    M = A_mem0.shape[1]
    _, H, DH = A_Wq.shape
    FH = B_w_in.shape[1] // 2
    seg = int(A_seg_len)
    big_rows = S // 2 + FH + S // 4 + FH // 2 + 13 * (FH // 4)
    out = pl.pallas_call(
        functools.partial(_kernel, seg=seg),
        out_shape=jax.ShapeDtypeStruct((S, D), A_x.dtype),
        in_specs=[pl.BlockSpec(memory_space=pl.ANY)] * 10,
        out_specs=pl.BlockSpec(memory_space=pl.ANY),
        scratch_shapes=[
            pltpu.VMEM((S, D), BF16),
            pltpu.VMEM((M, D), BF16),
            pltpu.VMEM((H // 2, 3, D, DH), U32),
            pltpu.VMEM((H, D // 2, 3 * DH), U32),
            pltpu.VMEM((H * DH // 2, D), U32),
            pltpu.VMEM((2, FH // 2, D), U32),
            pltpu.VMEM((big_rows, S), U32),
            pltpu.VMEM((S // LANES, LANES), BF16),
            pltpu.VMEM((FH // 2, D), U32),
            pltpu.VMEM((S // 2, D), U32),
            pltpu.VMEM((S // 2, FH), U32),
            pltpu.VMEM((M + seg, H * DH), F32),
            pltpu.VMEM((S, D), BF16),
            pltpu.SemaphoreType.DMA((20,)),
            pltpu.SemaphoreType.DMA(()),
        ],
        compiler_params=pltpu.CompilerParams(vmem_limit_bytes=120 * 1024 * 1024, disable_bounds_checks=True),
    )(
        A_x.reshape(S, D), A_mem0.reshape(M, D),
        *[w.reshape(D, H // 2, 2, DH) for w in (A_Wq, A_Wk, A_Wv)],
        A_Wo.reshape(H * DH, D), B_w_in.T, B_w_sp, B_b_sp.reshape(S // LANES, LANES), B_w_out,
    )
    return out.reshape(B, S, D)
```

```python
import functools

import jax
import jax.numpy as jnp
from jax import lax
from jax.experimental import pallas as pl
from jax.experimental.pallas import tpu as pltpu

F32 = jnp.float32
BF16 = jnp.bfloat16
U32 = jnp.uint32
EPS = 1e-5
NT = (((1,), (1,)), ((), ()))

LANES = 128
KH = 256
KY, NY = 384, 256
MB = 144

LN_ROWS = 16
PACK_ROWS = 16
FEED_LN, FEED_FINISH, FEED_PACK = 2, 4, 13
LN_FILL, FINISH_FILL, PACK_FILL = (0.35, 0.6, 0.8), 0.9, 0.95
FIRST_COPIES = 56
QKV_WAIT_AT, REST_WAIT_AT = 18, 26
UNROLL, PEEL = 4, 2
O_GROUPS = (0, 4, 7, 13, 32)
EARLY_PRODUCTS = (1, 3, 4, 2, 0)


def _layernorm(x):
    m = jnp.mean(x, axis=-1, keepdims=True)
    d = x - m
    v = jnp.mean(d * d, axis=-1, keepdims=True)
    return d * lax.rsqrt(v + EPS)


def _gelu2(x):
    c = 0.7978845608028654
    return x + x * jnp.tanh(x * (c + (c * 0.044715) * (x * x)))


def _silu_of_half(y2):
    hy = 0.25 * y2
    return hy + hy * jnp.tanh(hy)


def _recip(l):
    r = pl.reciprocal(l, approx=True)
    return r + r * (1.0 - l * r)


def _pack(w):
    return pltpu.bitcast(w.astype(BF16), U32)


def _unpack(w32):
    return pltpu.bitcast(w32, BF16)


def _dot(a, b):
    return jnp.dot(a, b, preferred_element_type=F32)


def _dot_nt(a, b):
    return lax.dot_general(a, b, NT, preferred_element_type=F32)


def _vreg_sum(x):
    return jnp.sum(x.reshape(x.shape[0] // 8, 8, x.shape[1]), axis=0)


def _tile(v, rows, cols=LANES):
    return jnp.concatenate([jnp.concatenate([v] * (rows // 8), axis=0)] * (cols // LANES), axis=1)


def _after(val, dep):
    return jnp.where(dep * dep < 0.0, pltpu.bitcast(dep, val.dtype), val)


class _SideWork:
    def __init__(self, gens=(), pieces=0, slots=1):
        self.gens, self.rate, self.credit = list(gens), pieces / slots, 0.0
        for g in self.gens:
            next(g)

    def feed(self, m, k=1):
        for t in range(k):
            self.credit += self.rate
            while self.gens and self.credit >= 1.0:
                self.credit -= 1.0
                r = t * (m.shape[0] // 8) // k * 8
                try:
                    self.gens[0].send(m[r:r + 8, :LANES])
                except StopIteration:
                    self.gens.pop(0)

    def drain(self, m):
        while self.gens:
            self.credit += 1.0
            self.feed(m)


def _strassen_left(a):
    return (a[0][0] + a[1][1], a[1][0] + a[1][1], a[0][0], a[1][1],
            a[0][0] + a[0][1], a[1][0] - a[0][0], a[0][1] - a[1][1])


_RIGHT_TERMS = (((0, 0), (1, 1), 1), ((0, 0), None, 0), ((0, 1), (1, 1), -1), ((1, 0), (0, 0), -1),
                ((1, 1), None, 0), ((0, 0), (0, 1), 1), ((1, 0), (1, 1), 1))
_LEFT_SUMS = (0, 1, 4, 5, 6)
_RIGHT_SUMS = (0, 2, 3, 5, 6)


def _strassen_right(p, b):
    first, second, sign = _RIGHT_TERMS[p]
    if second is None:
        return b(*first)
    return b(*first) + b(*second) if sign > 0 else b(*first) - b(*second)


def _strassen_combine(product, add, sub, done=lambda i, n, c: c, plain_left_first=False):
    if plain_left_first:
        m3, m4, m5 = product(2), product(3), product(4)
        c12 = done(0, 1, add(m3, m5))
        m2 = product(1)
        c21 = done(1, 0, add(m2, m4))
    else:
        m2, m4 = product(1), product(3)
        c21 = done(1, 0, add(m2, m4))
        m5, m3 = product(4), product(2)
        c12 = done(0, 1, add(m3, m5))
    d1, d2 = sub(m4, m5), sub(m3, m2)
    m1 = product(0)
    d1, d2 = add(d1, m1), add(d2, m1)
    c11 = done(0, 0, add(d1, product(6)))
    c22 = done(1, 1, add(d2, product(5)))
    return (c11, c12), (c21, c22)


def _segment_ops(heads):
    groups = [("O", a, b) for a, b in zip(O_GROUPS[:-1], O_GROUPS[1:])]
    ops = []
    for t in range(heads):
        ops.append(("P", t))
        if t >= 1:
            ops.append(("S", t - 1))
        if t >= 3:
            ops.append(("V", t - 3))
        if t == groups[0][2] + 3:
            ops.append(groups[0])
    ops += [groups[1], ("S", heads - 1), ("V", heads - 3), groups[2], ("V", heads - 2), ("V", heads - 1)]
    return ops + groups[3:]


def _gating_branch(x_hbm, mem_hbm, wq_hbm, wk_hbm, wv_hbm, wo_hbm, wint_hbm, wsp_hbm, bsp_hbm, wout_hbm,
                   x_v, mem_v, stage_v, wqkv_v, wo_v, wint_v, big_v, bsp_v, wout_v, wsum_v, xn_v, u_v, sem):
    S, D = x_v.shape
    heads, DH = wqkv_v.shape[0], wqkv_v.shape[2] // 3
    FH = u_v.shape[1]
    HS, QS = S // 2, S // 4
    HF, QF = FH // 2, FH // 4
    NB = QS // LANES
    n_sem = [0]

    def copy(src, dst):
        n_sem[0] += 1
        return pltpu.make_async_copy(src, dst, sem.at[n_sem[0]])

    def start(cps):
        for cp in cps:
            cp.start()

    def wait(cps):
        for cp in cps:
            cp.wait()

    def x_copies(a, b):
        rs = [slice(q * QS + a * LANES, q * QS + b * LANES) for q in range(4)]
        return [copy(x_hbm.at[r], x_v.at[r]) for r in rs]

    x0_cps, x1_cps, x2_cps = x_copies(0, 1), x_copies(1, 2), x_copies(2, NB)
    w1_cp = copy(wint_hbm.bitcast(U32).at[:HF], wint_v.at[0])

    def w2_copies(a, b):
        rs = [slice((i * HF + a) // 2, (i * HF + b) // 2) for i in range(2)]
        return [copy(wint_hbm.bitcast(U32).at[HF + r.start:HF + r.stop], wint_v.at[1, r]) for r in rs]

    w2a_cps, w2b_cps = w2_copies(0, MB), w2_copies(MB, HF)
    bsp_cp = copy(bsp_hbm, bsp_v)
    wsp_cp = copy(wsp_hbm.bitcast(U32), big_v.at[:HS])
    late_cps = [copy(mem_hbm, mem_v), copy(wout_hbm.bitcast(U32), wout_v), copy(wo_hbm.bitcast(U32), wo_v)]
    qkv_cps = [pltpu.make_async_copy(w.bitcast(U32).at[:, odd, hp, 0], stage_v.at[hp, j, odd], sem.at[0])
               for hp in range(heads // 2) for j, w in enumerate((wq_hbm, wk_hbm, wv_hbm)) for odd in range(2)]

    ZT = HS
    XS = ZT + FH
    WS = XS + HS // 2
    LF = WS + HF

    def tok(q, j, base=0):
        r = base + (q * QS + j * LANES) // 2
        return slice(r, r + LANES // 2)

    def cols(q, j):
        return slice(q * QS + j * LANES, q * QS + (j + 1) * LANES)

    def left_at(p, r0, r1, c0, c1):
        r = LF + (p // 4) * QF
        return slice(r + r0, r + r1), slice((p % 4) * QS + c0, (p % 4) * QS + c1)

    def ln_x(r, n, dep=None):
        xs = []
        for q in (r, HS + r):
            x = x_v[q:q + n, :].astype(F32)
            if dep is not None:
                x = jnp.concatenate([_after(x[:, :LANES], _tile(dep, n)), x[:, LANES:]], axis=1)
            xs.append(_layernorm(x))
            xn_v[q // 2:(q + n) // 2, :] = _pack(xs[-1])
        for i, p in enumerate(_RIGHT_SUMS):
            t = _strassen_right(p, lambda k, half: xs[half][:, k * KH:(k + 1) * KH])
            big_v[XS + r // 2:XS + (r + n) // 2, i * KH:(i + 1) * KH] = _pack(t)

    def ln_slices(j):
        for q in range(2):
            for r in range(q * QS + j * LANES, q * QS + (j + 1) * LANES, LN_ROWS):
                dep = yield
                ln_x(r, LN_ROWS, dep)

    def w_sums(which, a, b, dep=None):
        quad = [[_unpack(wint_v[which, (i * HF + a) // 2:(i * HF + b) // 2, k * KH:(k + 1) * KH]).astype(F32)
                 for k in range(2)] for i in range(2)]
        if dep is not None:
            dep = _tile(dep, b - a, KH)
            quad[0][0], quad[1][1] = _after(quad[0][0], dep), _after(quad[1][1], dep)
        left = _strassen_left(quad)
        r = WS + which * (HF // 2)
        for i, p in enumerate(_LEFT_SUMS):
            big_v[r + a // 2:r + b // 2, i * KH:(i + 1) * KH] = _pack(left[p])

    def w_sum_slices(which, a, b):
        for r in range(a, b, 16):
            dep = yield
            w_sums(which, r, r + 16, dep)

    def z_block(which, j, f, side, feed):
        tiles = [z_tile(which, j, q, f, side, feed) for q in range(2)]
        return [[jnp.concatenate([t[i][half] for t in tiles], axis=1) for half in range(2)] for i in range(2)]

    def z_tile(which, j, q, f, side, feed):
        def w(i, k):
            r = (i * HF + f) // 2
            return _unpack(wint_v[which, r:r + MB // 2, k * KH:min((k + 1) * KH, D)])

        def x(k, half):
            return _unpack(xn_v[tok(2 * half + q, j), k * KH:min((k + 1) * KH, D)])

        def left(p):
            if p not in _LEFT_SUMS:
                return w(p - 2, p - 2)
            i, r = _LEFT_SUMS.index(p), WS + (which * HF + f) // 2
            return _unpack(big_v[r:r + MB // 2, i * KH:(i + 1) * KH])

        def right(p):
            if p not in _RIGHT_SUMS:
                return x(p // 4, p // 4)
            i = _RIGHT_SUMS.index(p)
            return _unpack(big_v[tok(q, j, XS), i * KH:(i + 1) * KH])

        def dot(lhs, rhs):
            m = _dot_nt(lhs, rhs)
            side.feed(m, feed)
            return m

        return _strassen_combine(lambda p: dot(left(p), right(p)), jnp.add, jnp.subtract,
                                 lambda i, half, c: _gelu2(c + dot(w(i, 2), x(2, half))), plain_left_first=True)

    def finish_slices(j, sums, squares):
        ms, rs = [], []
        for half in range(2):
            m = jnp.sum(sums[half], axis=0, keepdims=True) * (1.0 / FH)
            v = jnp.maximum(jnp.sum(squares[half], axis=0, keepdims=True) * (1.0 / FH) - m * m, 0.0)
            r = lax.rsqrt(v + 4.0 * EPS)
            for q in range(2):
                ms.append(jnp.broadcast_to(m[:, q * LANES:(q + 1) * LANES], (8, LANES)))
                rs.append(jnp.broadcast_to(r[:, q * LANES:(q + 1) * LANES], (8, LANES)))
        for f in range(0, QF, 8):
            dep = yield
            mf = [_after(m, dep) for m in ms]
            a = [[(pltpu.bitcast(big_v[ZT + i * QF + f:ZT + i * QF + f + 8, cols(q, j)], F32) - mf[q]) * rs[q]
                  for q in range(4)] for i in range(4)]
            outer = [[_strassen_left([[a[2 * i + i2][2 * k + k2] for k in range(2)] for i in range(2)])
                      for k2 in range(2)] for i2 in range(2)]
            for p in range(7):
                quad = [[outer[i2][k2][p] for k2 in range(2)] for i2 in range(2)]
                if p:
                    dep = yield
                    quad[0][0], quad[1][1] = _after(quad[0][0], dep), _after(quad[1][1], dep)
                for p2, t in enumerate(_strassen_left(quad)):
                    big_v[left_at(7 * p + p2, f, f + 8, j * LANES, (j + 1) * LANES)] = pltpu.bitcast(t, U32)

    def repack_slices():
        low = jnp.full((8, DH), 0xFFFF, U32)
        for hp in range(heads // 2):
            for j in range(3):
                for r in range(0, D // 2, PACK_ROWS):
                    dep = yield
                    m = _tile(_after(low, dep), PACK_ROWS)
                    even, odd = (stage_v[hp, j, k, r:r + PACK_ROWS, :] for k in range(2))
                    wqkv_v[2 * hp, r:r + PACK_ROWS, j * DH:(j + 1) * DH] = (even & m) | (odd << 16)
                    wqkv_v[2 * hp + 1, r:r + PACK_ROWS, j * DH:(j + 1) * DH] = (even >> 16) | (odd & ~m)

    def wout_sum_slices():
        for i, p in enumerate(_RIGHT_SUMS):
            for r in range(0, KY // 2, 16):
                dep = yield
                assert issued[0] > REST_WAIT_AT, "w_out has not been waited for yet"
                t = _strassen_right(p, lambda k, n: _unpack(
                    wout_v[k * KY // 2 + r:k * KY // 2 + r + 16, n * NY:(n + 1) * NY]).astype(F32))
                wsum_v[i, r:r + 16, :] = _pack(_after(t, _tile(dep, 32, NY)))

    start(x0_cps[0::2] + x0_cps[1::2] + w2a_cps + w2b_cps + x1_cps)
    wait(x0_cps[0::2])
    ln_x(0, LANES)
    wait(x0_cps[1::2])
    ln_x(QS, LANES)
    wait(w2a_cps)
    w_sums(1, 0, MB)

    n_blocks = HF // MB
    products = 22
    ln_pieces = 2 * LANES // LN_ROWS
    finish_pieces = 7 * QF // 8

    side, finishes = _SideWork(), []
    for j in range(NB):
        sums, squares = [0.0, 0.0], [0.0, 0.0]
        for f in range(0, HF, MB):
            slots = (n_blocks - f // MB) * products
            if (j, f) == (0, MB):
                wait(w2b_cps)
                start(x2_cps + [bsp_cp, w1_cp, wsp_cp] + qkv_cps[:FIRST_COPIES])
                w_sums(1, MB, 2 * MB)
                side = _SideWork([w_sum_slices(1, 2 * MB, HF)], MB // 16, 0.7 * products * FEED_LN)
            if (j, f) == (0, 2 * MB):
                side.drain(partial)
                wait(x1_cps)
            if (j, f) == (1, MB):
                wait(x2_cps)
            if (j, f) in ((0, 2 * MB), (1, MB), (2, 0)):
                side = _SideWork([ln_slices(j + 1)], ln_pieces, LN_FILL[j] * slots * FEED_LN)
            if (j, f) == (NB - 1, 0):
                side = _SideWork([finishes.pop(0)], finish_pieces, FINISH_FILL * slots * FEED_FINISH)
            z = z_block(1, j, f, side, FEED_FINISH if j == NB - 1 else FEED_LN)
            for i in range(2):
                for half in range(2):
                    for q in range(2):
                        big_v[ZT + i * HF + f:ZT + i * HF + f + MB, cols(2 * half + q, j)] = pltpu.bitcast(
                            z[i][half][:, q * LANES:(q + 1) * LANES], U32)
                    partial = _vreg_sum(z[i][half])
                    sums[half] += partial
                    squares[half] += _vreg_sum(z[i][half] * z[i][half])
        side.drain(partial)
        finishes.append(finish_slices(j, sums, squares))
        if j == NB - 2:
            wait([bsp_cp, w1_cp])
            w_sums(0, 0, HF)

    side = _SideWork(finishes, len(finishes) * finish_pieces, FINISH_FILL * NB * n_blocks * products * FEED_FINISH)
    z1 = []
    for j in range(NB):
        z = [z_block(0, j, f, side, FEED_FINISH) for f in range(0, HF, MB)]
        z1.append([jnp.concatenate([blk[i][half] for i in range(2) for blk in z], axis=0) for half in range(2)])
    side.drain(z1[0][0])
    wsp_cp.wait()
    start(qkv_cps[FIRST_COPIES:] + late_cps)

    bias = bsp_v[...].astype(F32)
    issued, spatial_side = [0], [_SideWork()]

    def quadrantwise(op):
        return lambda a, b: [[op(a[i][n], b[i][n]) for n in range(2)] for i in range(2)]

    for j in range(NB):
        def outer_product(p):
            if issued[0] == REST_WAIT_AT:
                wait(late_cps)
            if issued[0] == QKV_WAIT_AT:
                pltpu.make_async_copy(stage_v, stage_v, sem.at[0]).wait()
                spatial_side[0] = _SideWork(
                    [repack_slices(), wout_sum_slices()], (heads // 2) * 3 * (D // 2 // PACK_ROWS) + 5 * KY // 32,
                    PACK_FILL * (7 * NB - QKV_WAIT_AT) * 7 * FEED_PACK)
            issued[0] += 1
            b = [[_strassen_right(p, lambda k, n: _unpack(
                big_v[tok(2 * n + n2, j), (2 * k + k2) * QS:(2 * k + k2 + 1) * QS]).astype(F32))
                for n2 in range(2)] for k2 in range(2)]

            def inner_product(p2):
                lhs = pltpu.bitcast(big_v[left_at(7 * p + p2, 0, QF, 0, QS)], F32)
                m = _dot_nt(lhs, _strassen_right(p2, lambda k, n: b[k][n]).astype(BF16))
                spatial_side[0].feed(m, FEED_PACK)
                return m

            return _strassen_combine(inner_product, jnp.add, jnp.subtract)

        c = _strassen_combine(outer_product, quadrantwise(jnp.add), quadrantwise(jnp.subtract))
        for half in range(2):
            g = jnp.concatenate(
                [jnp.concatenate([c[i][half][i2][q] for i in range(2) for i2 in range(2)], axis=0)
                 + bias[(2 * half + q) * NB + j:(2 * half + q) * NB + j + 1, :] for q in range(2)], axis=1)
            u = pltpu.bitcast((z1[j][half] * g).astype(BF16).T, U32)
            for q in range(2):
                u_v[tok(2 * half + q, j), :] = u[q * LANES // 2:(q + 1) * LANES // 2]
    spatial_side[0].drain(g)


def _recurrence(out_hbm, x_v, mem_v, wqkv_v, wo_v, wout_v, wsum_v, xn_v, u_v, o_v, out_v, sem_out, seg):
    heads, DH = wqkv_v.shape[0], wqkv_v.shape[2] // 3
    M = mem_v.shape[0]
    n_seg = x_v.shape[0] // seg
    scale = DH ** -0.5
    row = lax.broadcasted_iota(jnp.int32, (M + seg, M + seg), 0)
    col = lax.broadcasted_iota(jnp.int32, (M + seg, M + seg), 1)
    ops = _segment_ops(heads)

    def rows(s, n):
        return pl.ds(s * n, n) if isinstance(s, int) else pl.ds(pl.multiple_of(s * n, n), n)

    def segment(s, mem, last=False):
        q0 = M if last else 0
        mask = ((row < M) | (row >= col))[q0:]
        h = jnp.concatenate([mem, _unpack(xn_v[rows(s, seg // 2), :]).astype(F32)], axis=0)
        q, kv, probs, acc = {}, {}, {}, None
        for op, a, *rest in ops:
            if op == "P":
                if last:
                    q[a] = _dot(h[q0:], _unpack(wqkv_v[a, :, :DH]))
                    kv[a] = _dot(h, _unpack(wqkv_v[a, :, DH:]))
                else:
                    qkv = _dot(h, _unpack(wqkv_v[a]))
                    q[a], kv[a] = qkv[:, :DH], qkv[:, DH:]
            elif op == "S":
                scores = jnp.where(mask, _dot_nt(q.pop(a), kv[a][:, :DH]) * scale, -1e9)
                e = jnp.exp(scores - jnp.max(scores, axis=-1, keepdims=True))
                probs[a] = e, _recip(jnp.sum(e, axis=-1, keepdims=True))
            elif op == "V":
                e, inv = probs.pop(a)
                o_v[q0:, a * DH:(a + 1) * DH] = _dot(e, kv.pop(a)[:, DH:]) * inv
            else:
                b = rest[0]
                part = _dot(o_v[q0:, a * DH:b * DH], _unpack(wo_v[a * DH // 2:b * DH // 2, :]))
                acc = part if acc is None else acc + part
        return acc[:M, :], acc[M - q0:, :]

    def segment_pair(s, mem, followed, last=False):
        u = _unpack(u_v[rows(s // 2, seg), :])
        left = _strassen_left([[u[i * seg:(i + 1) * seg, k * KY:(k + 1) * KY].astype(F32) for k in range(2)]
                               for i in range(2)])

        def product(p):
            if p in _RIGHT_SUMS:
                return _dot(left[p], _unpack(wsum_v[_RIGHT_SUMS.index(p)]))
            k = p // 4
            return _dot(left[p], _unpack(wout_v[k * KY // 2:(k + 1) * KY // 2, k * NY:(k + 1) * NY]))

        def gate(early):
            c = _strassen_combine(lambda p: early[p] if p in early else product(p), jnp.add, jnp.subtract)
            return _silu_of_half(jnp.concatenate(
                [jnp.concatenate([jnp.concatenate(r, axis=1) for r in c], axis=0)
                 + _dot(u[:, 2 * KY:], _unpack(wout_v[KY:, :2 * NY])),
                 _dot(u, _unpack(wout_v[:, 2 * NY:]))], axis=1))

        mem, first = segment(s, mem)
        early = {p: product(p) for p in EARLY_PRODUCTS}
        g = None if followed else gate(early)
        mem, second = segment(s + 1, mem, last)
        g = gate(early) if followed else g
        r = rows(s // 2, 2 * seg)
        out_v[r, :] = (x_v[r, :].astype(F32) + jnp.concatenate([first, second], axis=0) * g).astype(out_v.dtype)
        pltpu.make_async_copy(out_v.at[r], out_hbm.at[r], sem_out).start()
        return mem

    def body(i, mem):
        for k in range(0, UNROLL, 2):
            mem = segment_pair(PEEL + i * UNROLL + k, mem, followed=k + 2 < UNROLL)
        return mem

    n_loop = n_seg // UNROLL - 1
    mem = mem_v[...].astype(F32)
    for s in range(0, PEEL, 2):
        mem = segment_pair(s, mem, followed=s + 2 < PEEL)
    mem = lax.fori_loop(0, n_loop, body, mem)
    for s in range(PEEL + n_loop * UNROLL, n_seg, 2):
        mem = segment_pair(s, mem, followed=s + 2 < n_seg, last=s + 2 == n_seg)
    pltpu.make_async_copy(out_v, out_hbm, sem_out).wait()


def _kernel(x_hbm, mem_hbm, wq_hbm, wk_hbm, wv_hbm, wo_hbm, wint_hbm, wsp_hbm, bsp_hbm, wout_hbm, out_hbm,
            x_v, mem_v, stage_v, wqkv_v, wo_v, wint_v, big_v, bsp_v, wout_v, wsum_v, xn_v, u_v, o_v, out_v,
            sem, sem_out, *, seg):
    _gating_branch(x_hbm, mem_hbm, wq_hbm, wk_hbm, wv_hbm, wo_hbm, wint_hbm, wsp_hbm, bsp_hbm, wout_hbm,
                   x_v, mem_v, stage_v, wqkv_v, wo_v, wint_v, big_v, bsp_v, wout_v, wsum_v, xn_v, u_v, sem)
    _recurrence(out_hbm, x_v, mem_v, wqkv_v, wo_v, wout_v, wsum_v, xn_v, u_v, o_v, out_v, sem_out, seg)


@functools.partial(jax.jit, static_argnames=("A_seg_len",))
def pallas_recurrent_scan__memory_aug_recurrent_mem_tr__mixer_gmlp__prompt_kernel(
    A_x, A_mem0, A_Wq, A_Wk, A_Wv, A_Wo, A_seg_len, B_x, B_w_in, B_w_sp, B_b_sp, B_w_out,
):
    del B_x
    B, S, D = A_x.shape
    M = A_mem0.shape[1]
    _, H, DH = A_Wq.shape
    FH = B_w_in.shape[1] // 2
    seg = int(A_seg_len)
    assert B == 1 and DH == LANES and S == 16 * LANES and H == O_GROUPS[-1]
    assert D == 2 * KH + LANES == 2 * NY + LANES and FH == 6 * MB and 2 * KY < FH
    big_rows = S // 2 + FH + S // 4 + FH // 2 + 13 * (FH // 4)
    out = pl.pallas_call(
        functools.partial(_kernel, seg=seg),
        out_shape=jax.ShapeDtypeStruct((S, D), A_x.dtype),
        in_specs=[pl.BlockSpec(memory_space=pl.ANY)] * 10,
        out_specs=pl.BlockSpec(memory_space=pl.ANY),
        scratch_shapes=[
            pltpu.VMEM((S, D), BF16),
            pltpu.VMEM((M, D), BF16),
            pltpu.VMEM((H // 2, 3, 2, D // 2, DH), U32),
            pltpu.VMEM((H, D // 2, 3 * DH), U32),
            pltpu.VMEM((H * DH // 2, D), U32),
            pltpu.VMEM((2, FH // 2, D), U32),
            pltpu.VMEM((big_rows, S), U32),
            pltpu.VMEM((S // LANES, LANES), BF16),
            pltpu.VMEM((FH // 2, D), U32),
            pltpu.VMEM((5, KY // 2, NY), U32),
            pltpu.VMEM((S // 2, D), U32),
            pltpu.VMEM((S // 2, FH), U32),
            pltpu.VMEM((M + seg, H * DH), F32),
            pltpu.VMEM((S, D), BF16),
            pltpu.SemaphoreType.DMA((24,)),
            pltpu.SemaphoreType.DMA(()),
        ],
        compiler_params=pltpu.CompilerParams(vmem_limit_bytes=120 * 1024 * 1024, disable_bounds_checks=True),
    )(
        A_x.reshape(S, D), A_mem0.reshape(M, D),
        *[w.reshape(D // 2, 2, H // 2, 2, DH) for w in (A_Wq, A_Wk, A_Wv)],
        A_Wo.reshape(H * DH, D), B_w_in.T, B_w_sp, B_b_sp.reshape(S // LANES, LANES), B_w_out,
    )
    return out.reshape(B, S, D)
```

```python
import functools

import jax
import jax.numpy as jnp
from jax import lax
from jax.experimental import pallas as pl
from jax.experimental.pallas import tpu as pltpu

F32 = jnp.float32
BF16 = jnp.bfloat16
U32 = jnp.uint32
EPS = 1e-5
NT = (((1,), (1,)), ((), ()))

LANES = 128
KH = 256
KY, NY = 384, 256
MB = 144
LATE = 8

LN_ROWS = 16
PACK_ROWS = 16
FEED_LN, FEED_FINISH, FEED_PACK = 2, 4, 13
LN_FILL, FINISH_FILL, PACK_FILL = (0.35, 0.6, 0.8), 0.9, 0.95
FIRST_COPIES = 56
QKV_WAIT_AT, REST_WAIT_AT = 18, 26
O_GROUPS = (0, 2, 5, 11, 32)
EARLY_PRODUCTS = (1, 3, 4, 2)
FACTOR_COLS, FACTOR_FILL = 256, 0.85
KV_PEEL, KV_LOOP = 2, 2


def _layernorm(x):
    m = jnp.mean(x, axis=-1, keepdims=True)
    d = x - m
    v = jnp.mean(d * d, axis=-1, keepdims=True)
    return d * lax.rsqrt(v + EPS)


def _gelu2(x):
    c = 0.7978845608028654
    return x + x * jnp.tanh(x * (c + (c * 0.044715) * (x * x)))


def _silu_of_half(y2):
    hy = 0.25 * y2
    return hy + hy * jnp.tanh(hy)


def _recip(l):
    r = pl.reciprocal(l, approx=True)
    return r + r * (1.0 - l * r)


def _pack(w):
    return pltpu.bitcast(w.astype(BF16), U32)


def _unpack(w32):
    return pltpu.bitcast(w32, BF16)


def _dot(a, b):
    return jnp.dot(a, b, preferred_element_type=F32)


def _dot_nt(a, b):
    return lax.dot_general(a, b, NT, preferred_element_type=F32)


def _vreg_sum(x):
    return jnp.sum(x.reshape(x.shape[0] // 8, 8, x.shape[1]), axis=0)


def _tile(v, rows, cols=LANES):
    return jnp.concatenate([jnp.concatenate([v] * (rows // 8), axis=0)] * (cols // LANES), axis=1)


def _after(val, dep):
    return jnp.where(dep * dep < 0.0, pltpu.bitcast(dep, val.dtype), val)


class _SideWork:
    def __init__(self, gens=(), pieces=0, slots=1):
        self.gens, self.rate, self.credit = list(gens), pieces / slots, 0.0
        for g in self.gens:
            next(g)

    def feed(self, m, k=1):
        for t in range(k):
            self.credit += self.rate
            while self.gens and self.credit >= 1.0:
                self.credit -= 1.0
                r = t * (m.shape[0] // 8) // k * 8
                try:
                    self.gens[0].send(m[r:r + 8, :LANES])
                except StopIteration:
                    self.gens.pop(0)

    def drain(self, m):
        while self.gens:
            self.credit += 1.0
            self.feed(m)


def _strassen_left(a):
    return (a[0][0] + a[1][1], a[1][0] + a[1][1], a[0][0], a[1][1],
            a[0][0] + a[0][1], a[1][0] - a[0][0], a[0][1] - a[1][1])


_RIGHT_TERMS = (((0, 0), (1, 1), 1), ((0, 0), None, 0), ((0, 1), (1, 1), -1), ((1, 0), (0, 0), -1),
                ((1, 1), None, 0), ((0, 0), (0, 1), 1), ((1, 0), (1, 1), 1))
_LEFT_SUMS = (0, 1, 4, 5, 6)
_RIGHT_SUMS = (0, 2, 3, 5, 6)


def _strassen_right(p, b):
    first, second, sign = _RIGHT_TERMS[p]
    if second is None:
        return b(*first)
    return b(*first) + b(*second) if sign > 0 else b(*first) - b(*second)


def _strassen_combine(product, add, sub, done=lambda i, n, c: c, plain_left_first=False):
    if plain_left_first:
        m3, m4, m5 = product(2), product(3), product(4)
        c12 = done(0, 1, add(m3, m5))
        m2 = product(1)
        c21 = done(1, 0, add(m2, m4))
    else:
        m2, m4 = product(1), product(3)
        c21 = done(1, 0, add(m2, m4))
        m5, m3 = product(4), product(2)
        c12 = done(0, 1, add(m3, m5))
    d1, d2 = sub(m4, m5), sub(m3, m2)
    m1 = product(0)
    d1, d2 = add(d1, m1), add(d2, m1)
    c11 = done(0, 0, add(d1, product(6)))
    c22 = done(1, 1, add(d2, product(5)))
    return (c11, c12), (c21, c22)


def _left_factors(a, emit):
    outer = [[_strassen_left([[a[2 * i + i2][2 * k + k2] for k in range(2)] for i in range(2)])
              for k2 in range(2)] for i2 in range(2)]
    for p in range(7):
        quad = [[outer[i2][k2][p] for k2 in range(2)] for i2 in range(2)]
        if p:
            dep = _tile((yield), *quad[0][0].shape)
            quad[0][0], quad[1][1] = _after(quad[0][0], dep), _after(quad[1][1], dep)
        for p2, t in enumerate(_strassen_left(quad)):
            emit(7 * p + p2, t)


def _strassen_squared(product, block, done=lambda i, n, c: c, before=lambda: None):
    c = [[None] * 4 for _ in range(4)]

    def quadrantwise(op):
        return lambda a, b: [[op(a[i][n], b[i][n]) for n in range(2)] for i in range(2)]

    add, sub = quadrantwise(jnp.add), quadrantwise(jnp.subtract)

    def outer(p, i=None, n=None, partial=None):
        def finish(i2, n2, t):
            c[2 * i + i2][2 * n + n2] = done(2 * i + i2, 2 * n + n2, partial[i2][n2] + t)
            return t

        before()
        b = [[_strassen_right(p, lambda k, m: block(2 * k + k2, 2 * m + n2).astype(F32))
              for n2 in range(2)] for k2 in range(2)]
        return _strassen_combine(
            lambda p2: product(7 * p + p2, _strassen_right(p2, lambda k, m: b[k][m]).astype(BF16)),
            jnp.add, jnp.subtract, finish if partial else lambda i2, n2, t: t)

    m2 = outer(1)
    m4 = outer(3, 1, 0, m2)
    m5 = outer(4)
    m3 = outer(2, 0, 1, m5)
    d1, d2 = sub(m4, m5), sub(m3, m2)
    m1 = outer(0)
    outer(6, 0, 0, add(d1, m1))
    outer(5, 1, 1, add(d2, m1))
    return c


def _segment_ops(heads):
    groups = [("O", a, b) for a, b in zip(O_GROUPS[:-1], O_GROUPS[1:])]
    ops = []
    for t in range(heads):
        ops.append(("P", t))
        if t >= 1:
            ops.append(("S", t - 1))
        if t >= 3:
            ops.append(("V", t - 3))
        if t == groups[0][2] + 3:
            ops.append(groups[0])
    ops += [groups[1], ("S", heads - 1), ("V", heads - 3), groups[2], ("V", heads - 2), ("V", heads - 1)]
    return ops + groups[3:]


def _gating_branch(x_hbm, mem_hbm, wq_hbm, wk_hbm, wv_hbm, wo_hbm, wint_hbm, wsp_hbm, bsp_hbm, wout_hbm,
                   x_v, mem_v, stage_v, wqkv_v, wo_v, wint_v, big_v, bsp_v, wout_v, wsum_v, xn_v, u_v, kv_v,
                   late_v, sem, seg):
    S, D = x_v.shape
    heads, DH = wqkv_v.shape[0], wqkv_v.shape[2] // 3
    FH = u_v.shape[1]
    HS, QS = S // 2, S // 4
    HF, QF = FH // 2, FH // 4
    NB = QS // LANES
    n_sem = [0]

    def copy(src, dst):
        n_sem[0] += 1
        return pltpu.make_async_copy(src, dst, sem.at[n_sem[0]])

    def start(cps):
        for cp in cps:
            cp.start()

    def wait(cps):
        for cp in cps:
            cp.wait()

    def x_copies(a, b):
        rs = [slice(q * QS + a * LANES, q * QS + b * LANES) for q in range(4)]
        return [copy(x_hbm.at[r], x_v.at[r]) for r in rs]

    x0_cps, x1_cps, x2_cps = x_copies(0, 1), x_copies(1, 2), x_copies(2, NB)
    w1_cp = copy(wint_hbm.bitcast(U32).at[:HF], wint_v.at[0])

    def w2_copies(a, b):
        rs = [slice((i * HF + a) // 2, (i * HF + b) // 2) for i in range(2)]
        return [copy(wint_hbm.bitcast(U32).at[HF + r.start:HF + r.stop], wint_v.at[1, r]) for r in rs]

    w2a_cps, w2b_cps = w2_copies(0, MB), w2_copies(MB, HF)
    bsp_cp = copy(bsp_hbm, bsp_v)
    wsp_cp = copy(wsp_hbm.bitcast(U32), big_v.at[:HS])
    late_cps = [copy(mem_hbm, mem_v), copy(wout_hbm.bitcast(U32), wout_v), copy(wo_hbm.bitcast(U32), wo_v)]
    qkv_cps = [pltpu.make_async_copy(w.bitcast(U32).at[:, odd, hp, 0], stage_v.at[hp, j, odd], sem.at[0])
               for hp in range(heads // 2) for j, w in enumerate((wq_hbm, wk_hbm, wv_hbm)) for odd in range(2)]

    ZT = HS
    XS = ZT + FH
    WS = XS + HS // 2
    LF = WS + HF
    XL = LF + 13 * QF
    KF = XL + 2 * LANES

    def tok(q, j, base=0):
        r = base + (q * QS + j * LANES) // 2
        return slice(r, r + LANES // 2)

    def cols(q, j):
        return slice(q * QS + j * LANES, q * QS + (j + 1) * LANES)

    def left_at(p, r0, r1, c0, c1):
        r = LF + (p // 4) * QF
        return slice(r + r0, r + r1), slice((p % 4) * QS + c0, (p % 4) * QS + c1)

    def late_at(q, r0, r1, c0, c1):
        r = XL + (q // 2) * LANES
        return slice(r + r0, r + r1), slice((q % 2) * D + c0, (q % 2) * D + c1)

    def kv_left_at(p, r0, r1):
        r = KF + (p // 16) * (LANES // 2)
        return slice(r + r0 // 2, r + r1 // 2), slice((p % 16) * LANES, (p % 16 + 1) * LANES)

    def ln_x(r, n, dep=None):
        xs = []
        for q in (r, HS + r):
            x = x_v[q:q + n, :].astype(F32)
            if dep is not None:
                x = jnp.concatenate([_after(x[:, :LANES], _tile(dep, n)), x[:, LANES:]], axis=1)
            xs.append(_layernorm(x))
            xn_v[q // 2:(q + n) // 2, :] = _pack(xs[-1])
            for t in range(q, q + n, LATE):
                if t % seg == seg - LATE:
                    g = t // seg // 4 * LATE
                    big_v[late_at(t // seg % 4, g, g + LATE, 0, D)] = pltpu.bitcast(xs[-1][t - q:t - q + LATE], U32)
        for i, p in enumerate(_RIGHT_SUMS):
            t = _strassen_right(p, lambda k, half: xs[half][:, k * KH:(k + 1) * KH])
            big_v[XS + r // 2:XS + (r + n) // 2, i * KH:(i + 1) * KH] = _pack(t)

    def ln_slices(j):
        for q in range(2):
            for r in range(q * QS + j * LANES, q * QS + (j + 1) * LANES, LN_ROWS):
                dep = yield
                ln_x(r, LN_ROWS, dep)

    def w_sums(which, a, b, dep=None):
        quad = [[_unpack(wint_v[which, (i * HF + a) // 2:(i * HF + b) // 2, k * KH:(k + 1) * KH]).astype(F32)
                 for k in range(2)] for i in range(2)]
        if dep is not None:
            dep = _tile(dep, b - a, KH)
            quad[0][0], quad[1][1] = _after(quad[0][0], dep), _after(quad[1][1], dep)
        left = _strassen_left(quad)
        r = WS + which * (HF // 2)
        for i, p in enumerate(_LEFT_SUMS):
            big_v[r + a // 2:r + b // 2, i * KH:(i + 1) * KH] = _pack(left[p])

    def w_sum_slices(which, a, b):
        for r in range(a, b, 16):
            dep = yield
            w_sums(which, r, r + 16, dep)

    def z_block(which, j, f, side, feed):
        tiles = [z_tile(which, j, q, f, side, feed) for q in range(2)]
        return [[jnp.concatenate([t[i][half] for t in tiles], axis=1) for half in range(2)] for i in range(2)]

    def z_tile(which, j, q, f, side, feed):
        def w(i, k):
            r = (i * HF + f) // 2
            return _unpack(wint_v[which, r:r + MB // 2, k * KH:min((k + 1) * KH, D)])

        def x(k, half):
            return _unpack(xn_v[tok(2 * half + q, j), k * KH:min((k + 1) * KH, D)])

        def left(p):
            if p not in _LEFT_SUMS:
                return w(p - 2, p - 2)
            i, r = _LEFT_SUMS.index(p), WS + (which * HF + f) // 2
            return _unpack(big_v[r:r + MB // 2, i * KH:(i + 1) * KH])

        def right(p):
            if p not in _RIGHT_SUMS:
                return x(p // 4, p // 4)
            i = _RIGHT_SUMS.index(p)
            return _unpack(big_v[tok(q, j, XS), i * KH:(i + 1) * KH])

        def dot(lhs, rhs):
            m = _dot_nt(lhs, rhs)
            side.feed(m, feed)
            return m

        return _strassen_combine(lambda p: dot(left(p), right(p)), jnp.add, jnp.subtract,
                                 lambda i, half, c: _gelu2(c + dot(w(i, 2), x(2, half))), plain_left_first=True)

    def finish_slices(j, sums, squares):
        ms, rs = [], []
        for half in range(2):
            m = jnp.sum(sums[half], axis=0, keepdims=True) * (1.0 / FH)
            v = jnp.maximum(jnp.sum(squares[half], axis=0, keepdims=True) * (1.0 / FH) - m * m, 0.0)
            r = lax.rsqrt(v + 4.0 * EPS)
            for q in range(2):
                ms.append(jnp.broadcast_to(m[:, q * LANES:(q + 1) * LANES], (8, LANES)))
                rs.append(jnp.broadcast_to(r[:, q * LANES:(q + 1) * LANES], (8, LANES)))
        for f in range(0, QF, 8):
            dep = yield
            mf = [_after(m, dep) for m in ms]
            a = [[(pltpu.bitcast(big_v[ZT + i * QF + f:ZT + i * QF + f + 8, cols(q, j)], F32) - mf[q]) * rs[q]
                  for q in range(4)] for i in range(4)]

            def emit(p, t):
                big_v[left_at(p, f, f + 8, j * LANES, (j + 1) * LANES)] = pltpu.bitcast(t, U32)

            yield from _left_factors(a, emit)

    def kv_left_slices():
        for r in range(0, LANES, 16):
            a = [[pltpu.bitcast(big_v[late_at(q, r, r + 16, k * LANES, (k + 1) * LANES)], F32) for k in range(4)]
                 for q in range(4)]

            def emit(p, t):
                big_v[kv_left_at(p, r, r + 16)] = _pack(t)

            yield from _left_factors(a, emit)

    def repack_slices():
        low = jnp.full((8, DH), 0xFFFF, U32)
        for hp in range(heads // 2):
            for j in range(3):
                for r in range(0, D // 2, PACK_ROWS):
                    dep = yield
                    m = _tile(_after(low, dep), PACK_ROWS)
                    even, odd = (stage_v[hp, j, k, r:r + PACK_ROWS, :] for k in range(2))
                    wqkv_v[2 * hp, r:r + PACK_ROWS, j * DH:(j + 1) * DH] = (even & m) | (odd << 16)
                    wqkv_v[2 * hp + 1, r:r + PACK_ROWS, j * DH:(j + 1) * DH] = (even >> 16) | (odd & ~m)

    def wout_sum_slices():
        for i, p in enumerate(_RIGHT_SUMS):
            for r in range(0, KY // 2, 16):
                dep = yield
                assert issued[0] > REST_WAIT_AT, "w_out has not been waited for yet"
                t = _strassen_right(p, lambda k, n: _unpack(
                    wout_v[k * KY // 2 + r:k * KY // 2 + r + 16, n * NY:(n + 1) * NY]).astype(F32))
                wsum_v[i, r:r + 16, :] = _pack(_after(t, _tile(dep, 32, NY)))

    start(x0_cps[0::2] + x0_cps[1::2] + w2a_cps + w2b_cps + x1_cps)
    late_v[...] = jnp.zeros(late_v.shape, F32)
    wait(x0_cps[0::2])
    ln_x(0, LANES)
    wait(x0_cps[1::2])
    ln_x(QS, LANES)
    wait(w2a_cps)
    w_sums(1, 0, MB)

    n_blocks = HF // MB
    products = 22
    ln_pieces = 2 * LANES // LN_ROWS
    finish_pieces = 7 * QF // 8

    side, finishes = _SideWork(), []
    for j in range(NB):
        sums, squares = [0.0, 0.0], [0.0, 0.0]
        for f in range(0, HF, MB):
            slots = (n_blocks - f // MB) * products
            if (j, f) == (0, MB):
                wait(w2b_cps)
                start(x2_cps + [bsp_cp, w1_cp, wsp_cp] + qkv_cps[:FIRST_COPIES])
                w_sums(1, MB, 2 * MB)
                side = _SideWork([w_sum_slices(1, 2 * MB, HF)], MB // 16, 0.7 * products * FEED_LN)
            if (j, f) == (0, 2 * MB):
                side.drain(partial)
                wait(x1_cps)
            if (j, f) == (1, MB):
                wait(x2_cps)
            if (j, f) in ((0, 2 * MB), (1, MB), (2, 0)):
                side = _SideWork([ln_slices(j + 1)], ln_pieces, LN_FILL[j] * slots * FEED_LN)
            if (j, f) == (NB - 1, 0):
                side = _SideWork([finishes.pop(0)], finish_pieces, FINISH_FILL * slots * FEED_FINISH)
            z = z_block(1, j, f, side, FEED_FINISH if j == NB - 1 else FEED_LN)
            for i in range(2):
                for half in range(2):
                    for q in range(2):
                        big_v[ZT + i * HF + f:ZT + i * HF + f + MB, cols(2 * half + q, j)] = pltpu.bitcast(
                            z[i][half][:, q * LANES:(q + 1) * LANES], U32)
                    partial = _vreg_sum(z[i][half])
                    sums[half] += partial
                    squares[half] += _vreg_sum(z[i][half] * z[i][half])
        side.drain(partial)
        finishes.append(finish_slices(j, sums, squares))
        if j == NB - 2:
            wait([bsp_cp, w1_cp])
            w_sums(0, 0, HF)

    side = _SideWork(finishes, len(finishes) * finish_pieces, FINISH_FILL * NB * n_blocks * products * FEED_FINISH)
    z1 = []
    for j in range(NB):
        z = [z_block(0, j, f, side, FEED_FINISH) for f in range(0, HF, MB)]
        z1.append([jnp.concatenate([blk[i][half] for i in range(2) for blk in z], axis=0) for half in range(2)])
    side.drain(z1[0][0])
    wsp_cp.wait()
    start(qkv_cps[FIRST_COPIES:] + late_cps)

    bias = bsp_v[...].astype(F32)
    issued, spatial_side = [0], [_SideWork([kv_left_slices()], 6 * LANES // 16, 0.9 * QKV_WAIT_AT * 7 * FEED_PACK)]

    def count_products():
        if issued[0] == REST_WAIT_AT:
            wait(late_cps)
        if issued[0] == QKV_WAIT_AT:
            assert not spatial_side[0].gens
            pltpu.make_async_copy(stage_v, stage_v, sem.at[0]).wait()
            spatial_side[0] = _SideWork(
                [repack_slices(), wout_sum_slices()], (heads // 2) * 3 * (D // 2 // PACK_ROWS) + 5 * KY // 32,
                PACK_FILL * (7 * NB - QKV_WAIT_AT) * 7 * FEED_PACK)
        issued[0] += 1

    def spatial_product(p, rhs):
        m = _dot_nt(pltpu.bitcast(big_v[left_at(p, 0, QF, 0, QS)], F32), rhs)
        spatial_side[0].feed(m, FEED_PACK)
        return m

    for j in range(NB):
        c = _strassen_squared(spatial_product, lambda k, n: _unpack(big_v[tok(n, j), k * QS:(k + 1) * QS]),
                              before=count_products)
        for half in range(2):
            g = jnp.concatenate(
                [jnp.concatenate([c[i][2 * half + q] for i in range(4)], axis=0)
                 + bias[(2 * half + q) * NB + j:(2 * half + q) * NB + j + 1, :] for q in range(2)], axis=1)
            u = pltpu.bitcast((z1[j][half] * g).astype(BF16).T, U32)
            for q in range(2):
                u_v[tok(2 * half + q, j), :] = u[q * LANES // 2:(q + 1) * LANES // 2]
    spatial_side[0].drain(g)

    def late_kv(a0):
        head = [a0 + n * (heads // 4) for n in range(4)]
        for j in (1, 2):
            c = _strassen_squared(
                lambda p, rhs: _dot(_unpack(big_v[kv_left_at(p, 0, LANES)]), rhs),
                lambda k, n: _unpack(wqkv_v[head[n], k * LANES // 2:(k + 1) * LANES // 2, j * DH:(j + 1) * DH]))
            x_rest = jnp.concatenate(
                [pltpu.bitcast(big_v[late_at(q, 0, LANES, 2 * KH, D)], F32) for q in range(4)], axis=0)
            for n in range(4):
                rest = _dot(x_rest, _unpack(wqkv_v[head[n], KH:, j * DH:(j + 1) * DH]))
                for pair in range(2):
                    kv_v[head[n], pair, :, (j - 1) * DH:j * DH] = pltpu.pack_elementwise(
                        [c[2 * pair + q][n] + rest[(2 * pair + q) * LANES:(2 * pair + q + 1) * LANES]
                         for q in range(2)], packed_dtype=BF16)

    per_step = (heads // 4 - KV_PEEL) // KV_LOOP
    for a0 in range(KV_PEEL):
        late_kv(a0)

    @pl.loop(0, KV_LOOP)
    def _(i):
        for a0 in range(per_step):
            late_kv(KV_PEEL + i * per_step + a0)


def _recurrence(out_hbm, x_v, mem_v, wqkv_v, wo_v, wout_v, wsum_v, big_v, xn_v, u_v, kv_v, late_v, o_v, out_v, sem_out,
                seg):
    heads, DH = wqkv_v.shape[0], wqkv_v.shape[2] // 3
    M, D = mem_v.shape
    n_groups = out_v.shape[0]
    early = seg - LATE
    KO = heads * DH // 4
    NO = 4 * LANES
    scale = DH ** -0.5
    row = lax.broadcasted_iota(jnp.int32, (M + seg, M + seg), 0)
    col = lax.broadcasted_iota(jnp.int32, (M + seg, M + seg), 1)
    ops = _segment_ops(heads)
    GL, XL, OF = 0, LANES, 2 * LANES

    def rows(i, n, base=0):
        return pl.ds(base + i * n, n) if isinstance(i, int) else pl.ds(pl.multiple_of(base + i * n, n), n)

    def copy_out(at):
        pltpu.make_async_copy(out_v.at[at], out_hbm.at[at], sem_out).start()

    def factor_slices(g):
        for t in range(0, KO, FACTOR_COLS):
            a = [[late_v[k, :, c * KO + t:c * KO + t + FACTOR_COLS] for c in range(4)] for k in range(4)]

            def emit(p, f):
                c0 = (p % 2) * KO + t
                big_v[rows(g, LATE, OF + p // 2 * LANES), c0:c0 + FACTOR_COLS] = pltpu.bitcast(f, U32)

            yield from _left_factors(a, emit)

    factor_pieces = 6 * KO // FACTOR_COLS

    def segment(g, k, mem, side, last):
        q0 = M if last else 0
        mask = ((row < M) | (row >= col))[q0:]
        h = jnp.concatenate([mem, _unpack(xn_v[rows(4 * g + k, seg // 2), :]).astype(F32)], axis=0)
        q, kv, probs, late, acc = {}, {}, {}, [], None
        for op, a, *rest in ops:
            if op == "P":
                q[a] = _dot(h[q0:], _unpack(wqkv_v[a, :, :DH]))
                side.feed(q[a], 2)
                kv[a] = jnp.concatenate(
                    [_dot(h[:M + early], _unpack(wqkv_v[a, :, DH:])),
                     pltpu.unpack_elementwise(kv_v[a, k // 2, rows(g, LATE), :], index=k % 2,
                                              packed_dtype=BF16, unpacked_dtype=F32)], axis=0)
            elif op == "S":
                scores = jnp.where(mask, _dot_nt(q.pop(a), kv[a][:, :DH]) * scale, -1e9)
                e = jnp.exp(scores - jnp.max(scores, axis=-1, keepdims=True))
                probs[a] = e, _recip(jnp.sum(e, axis=-1, keepdims=True))
            elif op == "V":
                e, inv = probs.pop(a)
                o = _dot(e, kv.pop(a)[:, DH:]) * inv
                o_v[q0:, a * DH:(a + 1) * DH] = o
                late.append(o[-LATE:])
                if a == heads - 1:
                    assert not side.gens, "the previous group's outputs are still being read"
                    late_v[k] = jnp.concatenate(late, axis=1)
                    if last:
                        side = _SideWork([factor_slices(g)], factor_pieces, 12)
            else:
                b = rest[0]
                w = slice(a * DH // 2, b * DH // 2)
                part = [_dot(o_v[q0:M + early, a * DH:b * DH], _unpack(wo_v[w, n:n + LANES]))
                        for n in range(0, NO, LANES)] + [_dot(o_v[q0:, a * DH:b * DH], _unpack(wo_v[w, NO:]))]
                acc = part if acc is None else [t + p for t, p in zip(acc, part)]
        for p in part[:4]:
            side.feed(p, 3)
        side.drain(part[3])
        out = jnp.concatenate(acc[:-1] + [acc[-1][:-LATE]], axis=1)
        return out[:M], out[M - q0:], acc[-1][-LATE:]

    def segment_pair(g, k, mem, followed, side, last=False):
        u = _unpack(u_v[rows(2 * g + k // 2, seg), :])
        left = _strassen_left([[u[i * seg:(i + 1) * seg, c * KY:(c + 1) * KY].astype(F32) for c in range(2)]
                               for i in range(2)])

        def product(p):
            if p in _RIGHT_SUMS:
                return _dot(left[p], _unpack(wsum_v[_RIGHT_SUMS.index(p)]))
            c = p // 4
            return _dot(left[p], _unpack(wout_v[c * KY // 2:(c + 1) * KY // 2, c * NY:(c + 1) * NY]))

        def gate(done):
            c = _strassen_combine(lambda p: done[p] if p in done else product(p), jnp.add, jnp.subtract)
            return _silu_of_half(jnp.concatenate(
                [jnp.concatenate([jnp.concatenate(r, axis=1) for r in c], axis=0)
                 + _dot(u[:, 2 * KY:], _unpack(wout_v[KY:, :2 * NY])),
                 _dot(u, _unpack(wout_v[:, 2 * NY:]))], axis=1))

        mem, *first = segment(g, k, mem, side, False)
        done = {p: product(p) for p in EARLY_PRODUCTS}
        gates = None if followed else gate(done)
        mem, *second = segment(g, k + 1, mem, side, last)
        gates = gate(done) if followed else gates
        for i, (attn, late_attn) in enumerate((first, second)):
            x = x_v[rows(4 * g + k + i, seg), :].astype(F32)
            gt = gates[i * seg:(i + 1) * seg]
            out_v[g, k + i, :early, :] = (x[:early] + attn * gt[:early]).astype(out_v.dtype)
            out_v[g, k + i, early:, NO:] = (x[early:, NO:] + late_attn * gt[early:, NO:]).astype(out_v.dtype)
            for base, t in ((GL, gt), (XL, x)):
                big_v[rows(g, LATE, base), (k + i) * NO:(k + i + 1) * NO] = pltpu.bitcast(t[early:, :NO], U32)
        return mem

    def group(g, mem, last=False):
        previous = g - 1 if last else jnp.maximum(g - 1, 0)
        side = _SideWork([factor_slices(previous)], factor_pieces, FACTOR_FILL * 2 * heads)
        mem = segment_pair(g, 0, mem, True, side)
        mem = segment_pair(g, 2, mem, False, side, last)
        if not last:
            copy_out((g, slice(None), slice(0, early)))
        return mem

    mem = lax.fori_loop(0, n_groups - 1, group, mem_v[...].astype(F32))
    group(n_groups - 1, mem, last=True)

    ready = [[], [], [(n_groups - 1, slice(None), slice(0, early)),
                  (slice(None), slice(None), slice(early, seg), slice(NO, D))]]

    def issue_copies():
        for at in ready.pop(0):
            copy_out(at)
        ready.append([])

    def late_output(k, n, c):
        t = slice(n * LANES, (n + 1) * LANES)
        gt, x = (pltpu.bitcast(big_v[base:base + LANES, k * NO + t.start:k * NO + t.stop], F32) for base in (GL, XL))
        out_v[:, k, early:, t] = (x + c * gt).reshape(n_groups, LATE, LANES).astype(out_v.dtype)
        ready[-1].append((slice(None), k, slice(early, seg), t))

    def late_product(p, rhs):
        issue_copies()
        return _dot(pltpu.bitcast(big_v[rows(p // 2, LANES, OF), (p % 2) * KO:(p % 2 + 1) * KO], F32), rhs)

    _strassen_squared(
        late_product, lambda k, n: _unpack(wo_v[k * KO // 2:(k + 1) * KO // 2, n * LANES:(n + 1) * LANES]), late_output)
    for _ in ready:
        issue_copies()
    pltpu.make_async_copy(out_v, out_hbm, sem_out).wait()


def _kernel(x_hbm, mem_hbm, wq_hbm, wk_hbm, wv_hbm, wo_hbm, wint_hbm, wsp_hbm, bsp_hbm, wout_hbm, out_hbm,
            x_v, mem_v, stage_v, wqkv_v, wo_v, wint_v, big_v, bsp_v, wout_v, wsum_v, xn_v, u_v, kv_v, late_v,
            o_v, out_v, sem, sem_out, *, seg):
    _gating_branch(x_hbm, mem_hbm, wq_hbm, wk_hbm, wv_hbm, wo_hbm, wint_hbm, wsp_hbm, bsp_hbm, wout_hbm,
                   x_v, mem_v, stage_v, wqkv_v, wo_v, wint_v, big_v, bsp_v, wout_v, wsum_v, xn_v, u_v, kv_v,
                   late_v, sem, seg)
    _recurrence(out_hbm, x_v, mem_v, wqkv_v, wo_v, wout_v, wsum_v, big_v, xn_v, u_v, kv_v, late_v, o_v, out_v,
                sem_out, seg)


@functools.partial(jax.jit, static_argnames=("A_seg_len",))
def pallas_recurrent_scan__memory_aug_recurrent_mem_tr__mixer_gmlp__prompt_kernel(
    A_x, A_mem0, A_Wq, A_Wk, A_Wv, A_Wo, A_seg_len, B_x, B_w_in, B_w_sp, B_b_sp, B_w_out,
):
    del B_x
    B, S, D = A_x.shape
    M = A_mem0.shape[1]
    _, H, DH = A_Wq.shape
    FH = B_w_in.shape[1] // 2
    seg = int(A_seg_len)
    assert B == 1 and DH == LANES and S == 16 * LANES and H == O_GROUPS[-1]
    assert D == 2 * KH + LANES == 2 * NY + LANES and FH == 6 * MB and 2 * KY < FH
    big_rows = S // 2 + FH + S // 4 + FH // 2 + 13 * (FH // 4) + 4 * LANES
    groups = (S // seg // 4, 4, seg, D)
    out = pl.pallas_call(
        functools.partial(_kernel, seg=seg),
        out_shape=jax.ShapeDtypeStruct(groups, A_x.dtype),
        in_specs=[pl.BlockSpec(memory_space=pl.ANY)] * 10,
        out_specs=pl.BlockSpec(memory_space=pl.ANY),
        scratch_shapes=[
            pltpu.VMEM((S, D), BF16),
            pltpu.VMEM((M, D), BF16),
            pltpu.VMEM((H // 2, 3, 2, D // 2, DH), U32),
            pltpu.VMEM((H, D // 2, 3 * DH), U32),
            pltpu.VMEM((H * DH // 2, D), U32),
            pltpu.VMEM((2, FH // 2, D), U32),
            pltpu.VMEM((big_rows, S), U32),
            pltpu.VMEM((S // LANES, LANES), BF16),
            pltpu.VMEM((FH // 2, D), U32),
            pltpu.VMEM((5, KY // 2, NY), U32),
            pltpu.VMEM((S // 2, D), U32),
            pltpu.VMEM((S // 2, FH), U32),
            pltpu.VMEM((H, 2, LANES, 2 * DH), U32),
            pltpu.VMEM((4, LATE, H * DH), F32),
            pltpu.VMEM((M + seg, H * DH), F32),
            pltpu.VMEM(groups, BF16),
            pltpu.SemaphoreType.DMA((24,)),
            pltpu.SemaphoreType.DMA(()),
        ],
        compiler_params=pltpu.CompilerParams(vmem_limit_bytes=126 * 1024 * 1024, disable_bounds_checks=True),
    )(
        A_x.reshape(S, D), A_mem0.reshape(M, D),
        *[w.reshape(D // 2, 2, H // 2, 2, DH) for w in (A_Wq, A_Wk, A_Wv)],
        A_Wo.reshape(H * DH, D), B_w_in.T, B_w_sp, B_b_sp.reshape(S // LANES, LANES), B_w_out,
    )
    return out.reshape(B, S, D)
```

```python
import functools

import jax
import jax.numpy as jnp
from jax import lax
from jax.experimental import pallas as pl
from jax.experimental.pallas import tpu as pltpu

F32 = jnp.float32
BF16 = jnp.bfloat16
U32 = jnp.uint32
EPS = 1e-5
NT = (((1,), (1,)), ((), ()))

LANES = 128
KH = 256
KY, NY = 384, 256
MB = 144
LATE = 8

LN_ROWS = 16
PACK_ROWS = 16
FEED_LN, FEED_FINISH, FEED_PACK = 2, 4, 13
LN_FILL, FINISH_FILL, PACK_FILL = (0.35, 0.6, 0.8), 0.9, 0.95
FIRST_COPIES = 56
QKV_WAIT_AT, REST_WAIT_AT = 18, 26
O_GROUPS = (0, 2, 5, 11, 32)
EARLY_PRODUCTS = (1, 3, 4, 2)
FACTOR_COLS, FACTOR_FILL = 256, 0.85
KV_PEEL, KV_LOOP = 2, 2


def _layernorm(x):
    m = jnp.mean(x, axis=-1, keepdims=True)
    d = x - m
    v = jnp.mean(d * d, axis=-1, keepdims=True)
    return d * lax.rsqrt(v + EPS)


def _gelu2(x):
    c = 0.7978845608028654
    return x + x * jnp.tanh(x * (c + (c * 0.044715) * (x * x)))


def _silu_of_half(y2):
    hy = 0.25 * y2
    return hy + hy * jnp.tanh(hy)


def _recip(l):
    r = pl.reciprocal(l, approx=True)
    return r + r * (1.0 - l * r)


def _pack(w):
    return pltpu.bitcast(w.astype(BF16), U32)


def _unpack(w32):
    return pltpu.bitcast(w32, BF16)


def _dot(a, b):
    return jnp.dot(a, b, preferred_element_type=F32)


def _dot_nt(a, b):
    return lax.dot_general(a, b, NT, preferred_element_type=F32)


def _vreg_sum(x):
    return jnp.sum(x.reshape(x.shape[0] // 8, 8, x.shape[1]), axis=0)


def _tile(v, rows, cols=LANES):
    return jnp.concatenate([jnp.concatenate([v] * (rows // 8), axis=0)] * (cols // LANES), axis=1)


def _after(val, dep):
    return jnp.where(dep * dep < 0.0, pltpu.bitcast(dep, val.dtype), val)


class _SideWork:
    def __init__(self, gens=(), pieces=0, slots=1):
        self.gens, self.rate, self.credit = list(gens), pieces / slots, 0.0
        for g in self.gens:
            next(g)

    def feed(self, m, k=1):
        for t in range(k):
            self.credit += self.rate
            while self.gens and self.credit >= 1.0:
                self.credit -= 1.0
                r = t * (m.shape[0] // 8) // k * 8
                try:
                    self.gens[0].send(m[r:r + 8, :LANES])
                except StopIteration:
                    self.gens.pop(0)

    def drain(self, m):
        while self.gens:
            self.credit += 1.0
            self.feed(m)


def _strassen_left(a):
    return (a[0][0] + a[1][1], a[1][0] + a[1][1], a[0][0], a[1][1],
            a[0][0] + a[0][1], a[1][0] - a[0][0], a[0][1] - a[1][1])


_RIGHT_TERMS = (((0, 0), (1, 1), 1), ((0, 0), None, 0), ((0, 1), (1, 1), -1), ((1, 0), (0, 0), -1),
                ((1, 1), None, 0), ((0, 0), (0, 1), 1), ((1, 0), (1, 1), 1))
_LEFT_SUMS = (0, 1, 4, 5, 6)
_RIGHT_SUMS = (0, 2, 3, 5, 6)


def _strassen_right(p, b):
    first, second, sign = _RIGHT_TERMS[p]
    if second is None:
        return b(*first)
    return b(*first) + b(*second) if sign > 0 else b(*first) - b(*second)


def _strassen_combine(product, add, sub, done=lambda i, n, c: c, plain_left_first=False):
    if plain_left_first:
        m3, m4, m5 = product(2), product(3), product(4)
        c12 = done(0, 1, add(m3, m5))
        m2 = product(1)
        c21 = done(1, 0, add(m2, m4))
    else:
        m2, m4 = product(1), product(3)
        c21 = done(1, 0, add(m2, m4))
        m5, m3 = product(4), product(2)
        c12 = done(0, 1, add(m3, m5))
    d1, d2 = sub(m4, m5), sub(m3, m2)
    m1 = product(0)
    d1, d2 = add(d1, m1), add(d2, m1)
    c11 = done(0, 0, add(d1, product(6)))
    c22 = done(1, 1, add(d2, product(5)))
    return (c11, c12), (c21, c22)


def _left_factors(a, emit):
    outer = [[_strassen_left([[a[2 * i + i2][2 * k + k2] for k in range(2)] for i in range(2)])
              for k2 in range(2)] for i2 in range(2)]
    for p in range(7):
        quad = [[outer[i2][k2][p] for k2 in range(2)] for i2 in range(2)]
        if p:
            dep = _tile((yield), *quad[0][0].shape)
            quad[0][0], quad[1][1] = _after(quad[0][0], dep), _after(quad[1][1], dep)
        for p2, t in enumerate(_strassen_left(quad)):
            emit(7 * p + p2, t)


def _strassen_squared(product, block, done=lambda i, n, c: c, before=lambda: None):
    c = [[None] * 4 for _ in range(4)]

    def quadrantwise(op):
        return lambda a, b: [[op(a[i][n], b[i][n]) for n in range(2)] for i in range(2)]

    add, sub = quadrantwise(jnp.add), quadrantwise(jnp.subtract)

    def outer(p, i=None, n=None, partial=None):
        def finish(i2, n2, t):
            c[2 * i + i2][2 * n + n2] = done(2 * i + i2, 2 * n + n2, partial[i2][n2] + t)
            return t

        before()
        b = [[_strassen_right(p, lambda k, m: block(2 * k + k2, 2 * m + n2).astype(F32))
              for n2 in range(2)] for k2 in range(2)]
        return _strassen_combine(
            lambda p2: product(7 * p + p2, _strassen_right(p2, lambda k, m: b[k][m]).astype(BF16)),
            jnp.add, jnp.subtract, finish if partial else lambda i2, n2, t: t)

    m2 = outer(1)
    m4 = outer(3, 1, 0, m2)
    m5 = outer(4)
    m3 = outer(2, 0, 1, m5)
    d1, d2 = sub(m4, m5), sub(m3, m2)
    m1 = outer(0)
    outer(6, 0, 0, add(d1, m1))
    outer(5, 1, 1, add(d2, m1))
    return c


def _segment_ops(heads):
    groups = [("O", a, b) for a, b in zip(O_GROUPS[:-1], O_GROUPS[1:])]
    ops = []
    for t in range(heads):
        ops += [(op, t - lag) for op, lag in (("P", 0), ("V", 3), ("S", 1)) if t >= lag]
        if t == groups[0][2] + 3:
            ops.append(groups[0])
    ops += [groups[1], ("S", heads - 1), ("V", heads - 3), groups[2], ("V", heads - 2), ("V", heads - 1)]
    return ops + groups[3:]


def _gating_branch(x_hbm, mem_hbm, wq_hbm, wk_hbm, wv_hbm, wo_hbm, wint_hbm, wsp_hbm, bsp_hbm, wout_hbm,
                   x_v, mem_v, stage_v, wqkv_v, wo_v, wint_v, big_v, bsp_v, wout_v, wsum_v, xn_v, u_v, kv_v,
                   late_v, sem, seg):
    S, D = x_v.shape
    heads, DH = wqkv_v.shape[0], wqkv_v.shape[2] // 3
    FH = u_v.shape[1]
    HS, QS = S // 2, S // 4
    HF, QF = FH // 2, FH // 4
    NB = QS // LANES
    n_sem = [0]

    def copy(src, dst):
        n_sem[0] += 1
        return pltpu.make_async_copy(src, dst, sem.at[n_sem[0]])

    def start(cps):
        for cp in cps:
            cp.start()

    def wait(cps):
        for cp in cps:
            cp.wait()

    def x_copies(a, b):
        rs = [slice(q * QS + a * LANES, q * QS + b * LANES) for q in range(4)]
        return [copy(x_hbm.at[r], x_v.at[r]) for r in rs]

    x0_cps, x1_cps, x2_cps = x_copies(0, 1), x_copies(1, 2), x_copies(2, NB)
    w1_cp = copy(wint_hbm.bitcast(U32).at[:HF], wint_v.at[0])

    def w2_copies(a, b):
        rs = [slice((i * HF + a) // 2, (i * HF + b) // 2) for i in range(2)]
        return [copy(wint_hbm.bitcast(U32).at[HF + r.start:HF + r.stop], wint_v.at[1, r]) for r in rs]

    w2a_cps, w2b_cps = w2_copies(0, MB), w2_copies(MB, HF)
    bsp_cp = copy(bsp_hbm, bsp_v)
    wsp_cp = copy(wsp_hbm.bitcast(U32), big_v.at[:HS])
    late_cps = [copy(mem_hbm, mem_v), copy(wout_hbm.bitcast(U32), wout_v), copy(wo_hbm.bitcast(U32), wo_v)]
    qkv_cps = [pltpu.make_async_copy(w.bitcast(U32).at[:, odd, hp, 0], stage_v.at[hp, j, odd], sem.at[0])
               for hp in range(heads // 2) for j, w in enumerate((wq_hbm, wk_hbm, wv_hbm)) for odd in range(2)]

    ZT = HS
    XS = ZT + FH
    WS = XS + HS // 2
    LF = WS + HF
    XL = LF + 13 * QF
    KF = XL + 2 * LANES

    def tok(q, j, base=0):
        r = base + (q * QS + j * LANES) // 2
        return slice(r, r + LANES // 2)

    def cols(q, j):
        return slice(q * QS + j * LANES, q * QS + (j + 1) * LANES)

    def left_at(p, r0, r1, c0, c1):
        r = LF + (p // 4) * QF
        return slice(r + r0, r + r1), slice((p % 4) * QS + c0, (p % 4) * QS + c1)

    def late_at(q, r0, r1, c0, c1):
        r = XL + (q // 2) * LANES
        return slice(r + r0, r + r1), slice((q % 2) * D + c0, (q % 2) * D + c1)

    def kv_left_at(p, r0, r1):
        r = KF + (p // 16) * (LANES // 2)
        return slice(r + r0 // 2, r + r1 // 2), slice((p % 16) * LANES, (p % 16 + 1) * LANES)

    def ln_x(r, n, dep=None):
        xs = []
        for q in (r, HS + r):
            x = x_v[q:q + n, :].astype(F32)
            if dep is not None:
                x = jnp.concatenate([_after(x[:, :LANES], _tile(dep, n)), x[:, LANES:]], axis=1)
            xs.append(_layernorm(x))
            xn_v[q // 2:(q + n) // 2, :] = _pack(xs[-1])
            for t in range(q, q + n, LATE):
                if t % seg == seg - LATE:
                    g = t // seg // 4 * LATE
                    big_v[late_at(t // seg % 4, g, g + LATE, 0, D)] = pltpu.bitcast(xs[-1][t - q:t - q + LATE], U32)
        for i, p in enumerate(_RIGHT_SUMS):
            t = _strassen_right(p, lambda k, half: xs[half][:, k * KH:(k + 1) * KH])
            big_v[XS + r // 2:XS + (r + n) // 2, i * KH:(i + 1) * KH] = _pack(t)

    def ln_slices(j):
        for q in range(2):
            for r in range(q * QS + j * LANES, q * QS + (j + 1) * LANES, LN_ROWS):
                dep = yield
                ln_x(r, LN_ROWS, dep)

    def w_sums(which, a, b, dep=None):
        quad = [[_unpack(wint_v[which, (i * HF + a) // 2:(i * HF + b) // 2, k * KH:(k + 1) * KH]).astype(F32)
                 for k in range(2)] for i in range(2)]
        if dep is not None:
            dep = _tile(dep, b - a, KH)
            quad[0][0], quad[1][1] = _after(quad[0][0], dep), _after(quad[1][1], dep)
        left = _strassen_left(quad)
        r = WS + which * (HF // 2)
        for i, p in enumerate(_LEFT_SUMS):
            big_v[r + a // 2:r + b // 2, i * KH:(i + 1) * KH] = _pack(left[p])

    def w_sum_slices(which, a, b):
        for r in range(a, b, 16):
            dep = yield
            w_sums(which, r, r + 16, dep)

    def z_block(which, j, f, side, feed):
        tiles = [z_tile(which, j, q, f, side, feed) for q in range(2)]
        return [[jnp.concatenate([t[i][half] for t in tiles], axis=1) for half in range(2)] for i in range(2)]

    def z_tile(which, j, q, f, side, feed):
        def w(i, k):
            r = (i * HF + f) // 2
            return _unpack(wint_v[which, r:r + MB // 2, k * KH:min((k + 1) * KH, D)])

        def x(k, half):
            return _unpack(xn_v[tok(2 * half + q, j), k * KH:min((k + 1) * KH, D)])

        def left(p):
            if p not in _LEFT_SUMS:
                return w(p - 2, p - 2)
            i, r = _LEFT_SUMS.index(p), WS + (which * HF + f) // 2
            return _unpack(big_v[r:r + MB // 2, i * KH:(i + 1) * KH])

        def right(p):
            if p not in _RIGHT_SUMS:
                return x(p // 4, p // 4)
            i = _RIGHT_SUMS.index(p)
            return _unpack(big_v[tok(q, j, XS), i * KH:(i + 1) * KH])

        def dot(lhs, rhs):
            m = _dot_nt(lhs, rhs)
            side.feed(m, feed)
            return m

        return _strassen_combine(lambda p: dot(left(p), right(p)), jnp.add, jnp.subtract,
                                 lambda i, half, c: _gelu2(c + dot(w(i, 2), x(2, half))), plain_left_first=True)

    def finish_slices(j, sums, squares):
        ms, rs = [], []
        for half in range(2):
            m = jnp.sum(sums[half], axis=0, keepdims=True) * (1.0 / FH)
            v = jnp.maximum(jnp.sum(squares[half], axis=0, keepdims=True) * (1.0 / FH) - m * m, 0.0)
            r = lax.rsqrt(v + 4.0 * EPS)
            for q in range(2):
                ms.append(jnp.broadcast_to(m[:, q * LANES:(q + 1) * LANES], (8, LANES)))
                rs.append(jnp.broadcast_to(r[:, q * LANES:(q + 1) * LANES], (8, LANES)))
        for f in range(0, QF, 8):
            dep = yield
            mf = [_after(m, dep) for m in ms]
            a = [[(pltpu.bitcast(big_v[ZT + i * QF + f:ZT + i * QF + f + 8, cols(q, j)], F32) - mf[q]) * rs[q]
                  for q in range(4)] for i in range(4)]

            def emit(p, t):
                big_v[left_at(p, f, f + 8, j * LANES, (j + 1) * LANES)] = pltpu.bitcast(t, U32)

            yield from _left_factors(a, emit)

    def kv_left_slices():
        for r in range(0, LANES, 16):
            a = [[pltpu.bitcast(big_v[late_at(q, r, r + 16, k * LANES, (k + 1) * LANES)], F32) for k in range(4)]
                 for q in range(4)]

            def emit(p, t):
                big_v[kv_left_at(p, r, r + 16)] = _pack(t)

            yield from _left_factors(a, emit)

    def repack_slices():
        low = jnp.full((8, DH), 0xFFFF, U32)
        for hp in range(heads // 2):
            for j in range(3):
                for r in range(0, D // 2, PACK_ROWS):
                    dep = yield
                    m = _tile(_after(low, dep), PACK_ROWS)
                    even, odd = (stage_v[hp, j, k, r:r + PACK_ROWS, :] for k in range(2))
                    wqkv_v[2 * hp, r:r + PACK_ROWS, j * DH:(j + 1) * DH] = (even & m) | (odd << 16)
                    wqkv_v[2 * hp + 1, r:r + PACK_ROWS, j * DH:(j + 1) * DH] = (even >> 16) | (odd & ~m)

    def wout_sum_slices():
        for i, p in enumerate(_RIGHT_SUMS):
            for r in range(0, KY // 2, 16):
                dep = yield
                assert issued[0] > REST_WAIT_AT, "w_out has not been waited for yet"
                t = _strassen_right(p, lambda k, n: _unpack(
                    wout_v[k * KY // 2 + r:k * KY // 2 + r + 16, n * NY:(n + 1) * NY]).astype(F32))
                wsum_v[i, r:r + 16, :] = _pack(_after(t, _tile(dep, 32, NY)))

    start(x0_cps[0::2] + x0_cps[1::2] + w2a_cps + w2b_cps + x1_cps)
    late_v[...] = jnp.zeros(late_v.shape, F32)
    wait(x0_cps[0::2])
    ln_x(0, LANES)
    wait(x0_cps[1::2])
    ln_x(QS, LANES)
    wait(w2a_cps)
    w_sums(1, 0, MB)

    n_blocks = HF // MB
    products = 22
    ln_pieces = 2 * LANES // LN_ROWS
    finish_pieces = 7 * QF // 8

    side, finishes = _SideWork(), []
    for j in range(NB):
        sums, squares = [0.0, 0.0], [0.0, 0.0]
        for f in range(0, HF, MB):
            slots = (n_blocks - f // MB) * products
            if (j, f) == (0, MB):
                wait(w2b_cps)
                start(x2_cps + [bsp_cp, w1_cp, wsp_cp] + qkv_cps[:FIRST_COPIES])
                w_sums(1, MB, 2 * MB)
                side = _SideWork([w_sum_slices(1, 2 * MB, HF)], MB // 16, 0.7 * products * FEED_LN)
            if (j, f) == (0, 2 * MB):
                side.drain(partial)
                wait(x1_cps)
            if (j, f) == (1, MB):
                wait(x2_cps)
            if (j, f) in ((0, 2 * MB), (1, MB), (2, 0)):
                side = _SideWork([ln_slices(j + 1)], ln_pieces, LN_FILL[j] * slots * FEED_LN)
            if (j, f) == (NB - 1, 0):
                side = _SideWork([finishes.pop(0)], finish_pieces, FINISH_FILL * slots * FEED_FINISH)
            z = z_block(1, j, f, side, FEED_FINISH if j == NB - 1 else FEED_LN)
            for i in range(2):
                for half in range(2):
                    for q in range(2):
                        big_v[ZT + i * HF + f:ZT + i * HF + f + MB, cols(2 * half + q, j)] = pltpu.bitcast(
                            z[i][half][:, q * LANES:(q + 1) * LANES], U32)
                    partial = _vreg_sum(z[i][half])
                    sums[half] += partial
                    squares[half] += _vreg_sum(z[i][half] * z[i][half])
        side.drain(partial)
        finishes.append(finish_slices(j, sums, squares))
        if j == NB - 2:
            wait([bsp_cp, w1_cp])
            w_sums(0, 0, HF)

    side = _SideWork(finishes, len(finishes) * finish_pieces, FINISH_FILL * NB * n_blocks * products * FEED_FINISH)
    z1 = []
    for j in range(NB):
        z = [z_block(0, j, f, side, FEED_FINISH) for f in range(0, HF, MB)]
        z1.append([jnp.concatenate([blk[i][half] for i in range(2) for blk in z], axis=0) for half in range(2)])
    side.drain(z1[0][0])
    wsp_cp.wait()
    start(qkv_cps[FIRST_COPIES:] + late_cps)

    bias = bsp_v[...].astype(F32)
    issued, spatial_side = [0], [_SideWork([kv_left_slices()], 6 * LANES // 16, 0.9 * QKV_WAIT_AT * 7 * FEED_PACK)]

    def count_products():
        if issued[0] == REST_WAIT_AT:
            wait(late_cps)
        if issued[0] == QKV_WAIT_AT:
            assert not spatial_side[0].gens
            pltpu.make_async_copy(stage_v, stage_v, sem.at[0]).wait()
            spatial_side[0] = _SideWork(
                [repack_slices(), wout_sum_slices()], (heads // 2) * 3 * (D // 2 // PACK_ROWS) + 5 * KY // 32,
                PACK_FILL * (7 * NB - QKV_WAIT_AT) * 7 * FEED_PACK)
        issued[0] += 1

    def spatial_product(p, rhs):
        m = _dot_nt(pltpu.bitcast(big_v[left_at(p, 0, QF, 0, QS)], F32), rhs)
        spatial_side[0].feed(m, FEED_PACK)
        return m

    for j in range(NB):
        c = _strassen_squared(spatial_product, lambda k, n: _unpack(big_v[tok(n, j), k * QS:(k + 1) * QS]),
                              before=count_products)
        for half in range(2):
            g = jnp.concatenate(
                [jnp.concatenate([c[i][2 * half + q] for i in range(4)], axis=0)
                 + bias[(2 * half + q) * NB + j:(2 * half + q) * NB + j + 1, :] for q in range(2)], axis=1)
            u = pltpu.bitcast((z1[j][half] * g).astype(BF16).T, U32)
            for q in range(2):
                u_v[tok(2 * half + q, j), :] = u[q * LANES // 2:(q + 1) * LANES // 2]
    spatial_side[0].drain(g)

    def late_kv(a0):
        head = [a0 + n * (heads // 4) for n in range(4)]
        for j in (1, 2):
            c = _strassen_squared(
                lambda p, rhs: _dot(_unpack(big_v[kv_left_at(p, 0, LANES)]), rhs),
                lambda k, n: _unpack(wqkv_v[head[n], k * LANES // 2:(k + 1) * LANES // 2, j * DH:(j + 1) * DH]))
            x_rest = jnp.concatenate(
                [pltpu.bitcast(big_v[late_at(q, 0, LANES, 2 * KH, D)], F32) for q in range(4)], axis=0)
            for n in range(4):
                rest = _dot(x_rest, _unpack(wqkv_v[head[n], KH:, j * DH:(j + 1) * DH]))
                for pair in range(2):
                    kv_v[head[n], pair, :, (j - 1) * DH:j * DH] = pltpu.pack_elementwise(
                        [c[2 * pair + q][n] + rest[(2 * pair + q) * LANES:(2 * pair + q + 1) * LANES]
                         for q in range(2)], packed_dtype=BF16)

    per_step = (heads // 4 - KV_PEEL) // KV_LOOP
    for a0 in range(KV_PEEL):
        late_kv(a0)

    @pl.loop(0, KV_LOOP)
    def _(i):
        for a0 in range(per_step):
            late_kv(KV_PEEL + i * per_step + a0)


def _recurrence(out_hbm, x_v, mem_v, wqkv_v, wo_v, wout_v, wsum_v, big_v, xn_v, u_v, kv_v, late_v, o_v, out_v, sem_out,
                seg):
    heads, DH = wqkv_v.shape[0], wqkv_v.shape[2] // 3
    M, D = mem_v.shape
    n_groups = out_v.shape[0]
    early = seg - LATE
    KO = heads * DH // 4
    NO = 4 * LANES
    scale = DH ** -0.5
    row = lax.broadcasted_iota(jnp.int32, (M + seg, M + seg), 0)
    col = lax.broadcasted_iota(jnp.int32, (M + seg, M + seg), 1)
    ops = _segment_ops(heads)
    GL, XL, OF = 0, LANES, 2 * LANES

    def rows(i, n, base=0):
        return pl.ds(base + i * n, n) if isinstance(i, int) else pl.ds(pl.multiple_of(base + i * n, n), n)

    def copy_out(at):
        pltpu.make_async_copy(out_v.at[at], out_hbm.at[at], sem_out).start()

    def factor_slices(g):
        for t in range(0, KO, FACTOR_COLS):
            a = [[late_v[k, :, c * KO + t:c * KO + t + FACTOR_COLS] for c in range(4)] for k in range(4)]

            def emit(p, f):
                c0 = (p % 2) * KO + t
                big_v[rows(g, LATE, OF + p // 2 * LANES), c0:c0 + FACTOR_COLS] = pltpu.bitcast(f, U32)

            yield from _left_factors(a, emit)

    factor_pieces = 6 * KO // FACTOR_COLS

    def segment(g, k, mem, side, last):
        q0 = M if last else 0
        mask = ((row < M) | (row >= col))[q0:]
        h = jnp.concatenate([mem, _unpack(xn_v[rows(4 * g + k, seg // 2), :]).astype(F32)], axis=0)
        q, kv, probs, late, acc = {}, {}, {}, [], None
        for op, a, *rest in ops:
            if op == "P":
                q[a] = _dot(h[q0:], _unpack(wqkv_v[a, :, :DH]))
                side.feed(q[a], 2)
                kv[a] = jnp.concatenate(
                    [_dot(h[:M + early], _unpack(wqkv_v[a, :, DH:])),
                     pltpu.unpack_elementwise(kv_v[a, k // 2, rows(g, LATE), :], index=k % 2,
                                              packed_dtype=BF16, unpacked_dtype=F32)], axis=0)
            elif op == "S":
                scores = jnp.where(mask, _dot_nt(q.pop(a), kv[a][:, :DH]) * scale, -1e9)
                e = jnp.exp(scores - jnp.max(scores, axis=-1, keepdims=True))
                probs[a] = e, _recip(jnp.sum(e, axis=-1, keepdims=True))
            elif op == "V":
                e, inv = probs.pop(a)
                o = _dot(e, kv.pop(a)[:, DH:]) * inv
                o_v[q0:, a * DH:(a + 1) * DH] = o
                late.append(o[-LATE:])
                if a == heads - 1:
                    assert not side.gens, "the previous group's outputs are still being read"
                    late_v[k] = jnp.concatenate(late, axis=1)
                    if last:
                        side = _SideWork([factor_slices(g)], factor_pieces, 12)
            else:
                b = rest[0]
                w = slice(a * DH // 2, b * DH // 2)
                part = [_dot(o_v[q0:M + early, a * DH:b * DH], _unpack(wo_v[w, n:n + LANES]))
                        for n in range(0, NO, LANES)] + [_dot(o_v[q0:, a * DH:b * DH], _unpack(wo_v[w, NO:]))]
                acc = part if acc is None else [t + p for t, p in zip(acc, part)]
        for p in part[:4]:
            side.feed(p, 3)
        side.drain(part[3])
        out = jnp.concatenate(acc[:-1] + [acc[-1][:-LATE]], axis=1)
        return out[:M], out[M - q0:], acc[-1][-LATE:]

    def segment_pair(g, k, mem, followed, side, last=False):
        u = _unpack(u_v[rows(2 * g + k // 2, seg), :])
        left = _strassen_left([[u[i * seg:(i + 1) * seg, c * KY:(c + 1) * KY].astype(F32) for c in range(2)]
                               for i in range(2)])

        def product(p):
            if p in _RIGHT_SUMS:
                return _dot(left[p], _unpack(wsum_v[_RIGHT_SUMS.index(p)]))
            c = p // 4
            return _dot(left[p], _unpack(wout_v[c * KY // 2:(c + 1) * KY // 2, c * NY:(c + 1) * NY]))

        def gate(done):
            c = _strassen_combine(lambda p: done[p] if p in done else product(p), jnp.add, jnp.subtract)
            return _silu_of_half(jnp.concatenate(
                [jnp.concatenate([jnp.concatenate(r, axis=1) for r in c], axis=0)
                 + _dot(u[:, 2 * KY:], _unpack(wout_v[KY:, :2 * NY])),
                 _dot(u, _unpack(wout_v[:, 2 * NY:]))], axis=1))

        mem, *first = segment(g, k, mem, side, False)
        done = {p: product(p) for p in EARLY_PRODUCTS}
        gates = None if followed else gate(done)
        mem, *second = segment(g, k + 1, mem, side, last)
        gates = gate(done) if followed else gates
        for i, (attn, late_attn) in enumerate((first, second)):
            x = x_v[rows(4 * g + k + i, seg), :].astype(F32)
            gt = gates[i * seg:(i + 1) * seg]
            out_v[g, k + i, :early, :] = (x[:early] + attn * gt[:early]).astype(out_v.dtype)
            out_v[g, k + i, early:, NO:] = (x[early:, NO:] + late_attn * gt[early:, NO:]).astype(out_v.dtype)
            for base, t in ((GL, gt), (XL, x)):
                big_v[rows(g, LATE, base), (k + i) * NO:(k + i + 1) * NO] = pltpu.bitcast(t[early:, :NO], U32)
        return mem

    def group(g, mem, last=False):
        previous = g - 1 if last else jnp.maximum(g - 1, 0)
        side = _SideWork([factor_slices(previous)], factor_pieces, FACTOR_FILL * 2 * heads)
        mem = segment_pair(g, 0, mem, True, side)
        mem = segment_pair(g, 2, mem, False, side, last)
        if not last:
            copy_out((g, slice(None), slice(0, early)))
        return mem

    mem = lax.fori_loop(0, n_groups - 1, group, mem_v[...].astype(F32))
    group(n_groups - 1, mem, last=True)

    ready = [[], [], [(n_groups - 1, slice(None), slice(0, early)),
                  (slice(None), slice(None), slice(early, seg), slice(NO, D))]]

    def issue_copies():
        for at in ready.pop(0):
            copy_out(at)
        ready.append([])

    def late_output(k, n, c):
        t = slice(n * LANES, (n + 1) * LANES)
        gt, x = (pltpu.bitcast(big_v[base:base + LANES, k * NO + t.start:k * NO + t.stop], F32) for base in (GL, XL))
        out_v[:, k, early:, t] = (x + c * gt).reshape(n_groups, LATE, LANES).astype(out_v.dtype)
        ready[-1].append((slice(None), k, slice(early, seg), t))

    def late_product(p, rhs):
        issue_copies()
        return _dot(pltpu.bitcast(big_v[rows(p // 2, LANES, OF), (p % 2) * KO:(p % 2 + 1) * KO], F32), rhs)

    _strassen_squared(
        late_product, lambda k, n: _unpack(wo_v[k * KO // 2:(k + 1) * KO // 2, n * LANES:(n + 1) * LANES]), late_output)
    for _ in ready:
        issue_copies()
    pltpu.make_async_copy(out_v, out_hbm, sem_out).wait()


def _kernel(x_hbm, mem_hbm, wq_hbm, wk_hbm, wv_hbm, wo_hbm, wint_hbm, wsp_hbm, bsp_hbm, wout_hbm, out_hbm,
            x_v, mem_v, stage_v, wqkv_v, wo_v, wint_v, big_v, bsp_v, wout_v, wsum_v, xn_v, u_v, kv_v, late_v,
            o_v, out_v, sem, sem_out, *, seg):
    _gating_branch(x_hbm, mem_hbm, wq_hbm, wk_hbm, wv_hbm, wo_hbm, wint_hbm, wsp_hbm, bsp_hbm, wout_hbm,
                   x_v, mem_v, stage_v, wqkv_v, wo_v, wint_v, big_v, bsp_v, wout_v, wsum_v, xn_v, u_v, kv_v,
                   late_v, sem, seg)
    _recurrence(out_hbm, x_v, mem_v, wqkv_v, wo_v, wout_v, wsum_v, big_v, xn_v, u_v, kv_v, late_v, o_v, out_v,
                sem_out, seg)


@functools.partial(jax.jit, static_argnames=("A_seg_len",))
def pallas_recurrent_scan__memory_aug_recurrent_mem_tr__mixer_gmlp__prompt_kernel(
    A_x, A_mem0, A_Wq, A_Wk, A_Wv, A_Wo, A_seg_len, B_x, B_w_in, B_w_sp, B_b_sp, B_w_out,
):
    del B_x
    B, S, D = A_x.shape
    M = A_mem0.shape[1]
    _, H, DH = A_Wq.shape
    FH = B_w_in.shape[1] // 2
    seg = int(A_seg_len)
    assert B == 1 and DH == LANES and S == 16 * LANES and H == O_GROUPS[-1]
    assert D == 2 * KH + LANES == 2 * NY + LANES and FH == 6 * MB and 2 * KY < FH
    big_rows = S // 2 + FH + S // 4 + FH // 2 + 13 * (FH // 4) + 4 * LANES
    groups = (S // seg // 4, 4, seg, D)
    out = pl.pallas_call(
        functools.partial(_kernel, seg=seg),
        out_shape=jax.ShapeDtypeStruct(groups, A_x.dtype),
        in_specs=[pl.BlockSpec(memory_space=pl.ANY)] * 10,
        out_specs=pl.BlockSpec(memory_space=pl.ANY),
        scratch_shapes=[
            pltpu.VMEM((S, D), BF16),
            pltpu.VMEM((M, D), BF16),
            pltpu.VMEM((H // 2, 3, 2, D // 2, DH), U32),
            pltpu.VMEM((H, D // 2, 3 * DH), U32),
            pltpu.VMEM((H * DH // 2, D), U32),
            pltpu.VMEM((2, FH // 2, D), U32),
            pltpu.VMEM((big_rows, S), U32),
            pltpu.VMEM((S // LANES, LANES), BF16),
            pltpu.VMEM((FH // 2, D), U32),
            pltpu.VMEM((5, KY // 2, NY), U32),
            pltpu.VMEM((S // 2, D), U32),
            pltpu.VMEM((S // 2, FH), U32),
            pltpu.VMEM((H, 2, LANES, 2 * DH), U32),
            pltpu.VMEM((4, LATE, H * DH), F32),
            pltpu.VMEM((M + seg, H * DH), F32),
            pltpu.VMEM(groups, BF16),
            pltpu.SemaphoreType.DMA((24,)),
            pltpu.SemaphoreType.DMA(()),
        ],
        compiler_params=pltpu.CompilerParams(vmem_limit_bytes=126 * 1024 * 1024, disable_bounds_checks=True),
    )(
        A_x.reshape(S, D), A_mem0.reshape(M, D),
        *[w.reshape(D // 2, 2, H // 2, 2, DH) for w in (A_Wq, A_Wk, A_Wv)],
        A_Wo.reshape(H * DH, D), B_w_in.T, B_w_sp, B_b_sp.reshape(S // LANES, LANES), B_w_out,
    )
    return out.reshape(B, S, D)
```

```python
import functools

import jax
import jax.numpy as jnp
from jax import lax
from jax.experimental import pallas as pl
from jax.experimental.pallas import tpu as pltpu

F32 = jnp.float32
BF16 = jnp.bfloat16
U32 = jnp.uint32
EPS = 1e-5
NT = (((1,), (1,)), ((), ()))

LANES = 128
KH = 256
KY, NY = 384, 256
MB = 144
LATE = 8

LN_ROWS = 16
PACK_ROWS = 16
FEED_LN, FEED_FINISH, FEED_PACK = 2, 4, 13
LN_FILL, FINISH_FILL, PACK_FILL = (0.35, 0.6, 0.8), 0.9, 0.98
FIRST_COPIES = 56
QKV_WAIT_AT, REST_WAIT_AT = 18, 26
S_LAG, V_LAG = 2, 5
O_GROUPS = (0, 2, 5, 11, 32)
EARLY_PRODUCTS = (1, 3, 4, 2)
FACTOR_COLS, FACTOR_FILL = 256, 0.85
QKV_LOOP = 2


def _layernorm(x):
    m = jnp.mean(x, axis=-1, keepdims=True)
    d = x - m
    v = jnp.mean(d * d, axis=-1, keepdims=True)
    return d * lax.rsqrt(v + EPS)


def _gelu2(x):
    c = 0.7978845608028654
    return x + x * jnp.tanh(x * (c + (c * 0.044715) * (x * x)))


def _silu_of_half(y2):
    hy = 0.25 * y2
    return hy + hy * jnp.tanh(hy)


def _recip(l):
    r = pl.reciprocal(l, approx=True)
    return r + r * (1.0 - l * r)


def _pack(w):
    return pltpu.bitcast(w.astype(BF16), U32)


def _unpack(w32):
    return pltpu.bitcast(w32, BF16)


def _dot(a, b):
    return jnp.dot(a, b, preferred_element_type=F32)


def _dot_nt(a, b):
    return lax.dot_general(a, b, NT, preferred_element_type=F32)


def _vreg_sum(x):
    return jnp.sum(x.reshape(x.shape[0] // 8, 8, x.shape[1]), axis=0)


def _rows(i, n, base=0):
    start = base + i * n
    return pl.ds(start if isinstance(i, int) else pl.multiple_of(start, n), n)


def _tile(v, rows, cols=LANES):
    return jnp.concatenate([jnp.concatenate([v] * (rows // 8), axis=0)] * (cols // LANES), axis=1)


def _after(val, dep):
    return jnp.where(dep * dep < 0.0, pltpu.bitcast(dep, val.dtype), val)


class _SideWork:
    def __init__(self, gens=(), pieces=0, slots=1):
        self.gens, self.rate, self.credit = list(gens), pieces / slots, 0.0
        for g in self.gens:
            next(g)

    def feed(self, m, k=1):
        for t in range(k):
            self.credit += self.rate
            while self.gens and self.credit >= 1.0:
                self.credit -= 1.0
                r = t * (m.shape[0] // 8) // k * 8
                try:
                    self.gens[0].send(m[r:r + 8, :LANES])
                except StopIteration:
                    self.gens.pop(0)

    def drain(self, m):
        while self.gens:
            self.credit += 1.0
            self.feed(m)


def _strassen_left(a):
    return (a[0][0] + a[1][1], a[1][0] + a[1][1], a[0][0], a[1][1],
            a[0][0] + a[0][1], a[1][0] - a[0][0], a[0][1] - a[1][1])


_RIGHT_TERMS = (((0, 0), (1, 1), 1), ((0, 0), None, 0), ((0, 1), (1, 1), -1), ((1, 0), (0, 0), -1),
                ((1, 1), None, 0), ((0, 0), (0, 1), 1), ((1, 0), (1, 1), 1))
_LEFT_SUMS = (0, 1, 4, 5, 6)
_RIGHT_SUMS = (0, 2, 3, 5, 6)


def _strassen_right(p, b):
    first, second, sign = _RIGHT_TERMS[p]
    if second is None:
        return b(*first)
    return b(*first) + b(*second) if sign > 0 else b(*first) - b(*second)


def _strassen_combine(product, add, sub, done=lambda i, n, c: c, plain_left_first=False):
    if plain_left_first:
        m3, m4, m5 = product(2), product(3), product(4)
        c12 = done(0, 1, add(m3, m5))
        m2 = product(1)
        c21 = done(1, 0, add(m2, m4))
    else:
        m2, m4 = product(1), product(3)
        c21 = done(1, 0, add(m2, m4))
        m5, m3 = product(4), product(2)
        c12 = done(0, 1, add(m3, m5))
    d1, d2 = sub(m4, m5), sub(m3, m2)
    m1 = product(0)
    d1, d2 = add(d1, m1), add(d2, m1)
    c11 = done(0, 0, add(d1, product(6)))
    c22 = done(1, 1, add(d2, product(5)))
    return (c11, c12), (c21, c22)


def _left_factors(a, emit):
    outer = [[_strassen_left([[a[2 * i + i2][2 * k + k2] for k in range(2)] for i in range(2)])
              for k2 in range(2)] for i2 in range(2)]
    for p in range(7):
        quad = [[outer[i2][k2][p] for k2 in range(2)] for i2 in range(2)]
        if p:
            dep = _tile((yield), *quad[0][0].shape)
            quad[0][0], quad[1][1] = _after(quad[0][0], dep), _after(quad[1][1], dep)
        for p2, t in enumerate(_strassen_left(quad)):
            emit(7 * p + p2, t)


def _strassen_squared(product, block, done=lambda i, n, c: c, before=lambda: None, dtype=F32):
    c = [[None] * 4 for _ in range(4)]

    def quadrantwise(op):
        return lambda a, b: [[op(a[i][n], b[i][n]) for n in range(2)] for i in range(2)]

    add, sub = quadrantwise(jnp.add), quadrantwise(jnp.subtract)

    def outer(p, i=None, n=None, partial=None):
        def finish(i2, n2, t):
            c[2 * i + i2][2 * n + n2] = done(2 * i + i2, 2 * n + n2, partial[i2][n2] + t)
            return t

        before()
        b = [[_strassen_right(p, lambda k, m: block(2 * k + k2, 2 * m + n2).astype(F32))
              for n2 in range(2)] for k2 in range(2)]
        return _strassen_combine(
            lambda p2: product(7 * p + p2, _strassen_right(p2, lambda k, m: b[k][m]).astype(dtype)),
            jnp.add, jnp.subtract, finish if partial else lambda i2, n2, t: t)

    m2 = outer(1)
    m4 = outer(3, 1, 0, m2)
    m5 = outer(4)
    m3 = outer(2, 0, 1, m5)
    d1, d2 = sub(m4, m5), sub(m3, m2)
    m1 = outer(0)
    outer(6, 0, 0, add(d1, m1))
    outer(5, 1, 1, add(d2, m1))
    return c


def _segment_ops(heads):
    groups = [("O", a, b) for a, b in zip(O_GROUPS[:-1], O_GROUPS[1:])]
    ops = []
    for t in range(heads):
        ops += [("P", t, j) for j in range(3)]
        ops += [(op, t - lag) for op, lag in (("V", V_LAG), ("S", S_LAG)) if t >= lag]
        if t == groups[0][2] + V_LAG:
            ops.append(groups[0])
    scores = [("S", a) for a in range(heads - S_LAG, heads)]
    values = [("V", a) for a in range(heads - V_LAG, heads)]
    return ops + [groups[1]] + scores + values[:1] + [groups[2]] + values[1:] + groups[3:]


def _gating_branch(x_hbm, mem_hbm, wq_hbm, wk_hbm, wv_hbm, wo_hbm, wint_hbm, wsp_hbm, bsp_hbm, wout_hbm,
                   x_v, mem_v, stage_v, wqkv_v, wo_v, wint_v, big_v, bsp_v, wout_v, wsum_v, xn_v, u_v, late_v,
                   sem, seg):
    S, D = x_v.shape
    heads, DH = wqkv_v.shape[0], wqkv_v.shape[2] // 3
    FH = u_v.shape[1]
    HS, QS = S // 2, S // 4
    HF, QF = FH // 2, FH // 4
    NB = QS // LANES
    n_sem = [0]

    def copy(src, dst):
        n_sem[0] += 1
        return pltpu.make_async_copy(src, dst, sem.at[n_sem[0]])

    def start(cps):
        for cp in cps:
            cp.start()

    def wait(cps):
        for cp in cps:
            cp.wait()

    def x_copies(a, b):
        rs = [slice(q * QS + a * LANES, q * QS + b * LANES) for q in range(4)]
        return [copy(x_hbm.at[r], x_v.at[r]) for r in rs]

    x0_cps, x1_cps, x2_cps = x_copies(0, 1), x_copies(1, 2), x_copies(2, NB)
    w1_cp = copy(wint_hbm.bitcast(U32).at[:HF], wint_v.at[0])

    def w2_copies(a, b):
        rs = [slice((i * HF + a) // 2, (i * HF + b) // 2) for i in range(2)]
        return [copy(wint_hbm.bitcast(U32).at[HF + r.start:HF + r.stop], wint_v.at[1, r]) for r in rs]

    w2a_cps, w2b_cps = w2_copies(0, MB), w2_copies(MB, HF)
    bsp_cp = copy(bsp_hbm, bsp_v)
    wsp_cp = copy(wsp_hbm.bitcast(U32), big_v.at[:HS])
    late_cps = [copy(mem_hbm, mem_v), copy(wout_hbm.bitcast(U32), wout_v), copy(wo_hbm.bitcast(U32), wo_v)]
    qkv_cps = [pltpu.make_async_copy(w.bitcast(U32).at[:, odd, hp, 0], stage_v.at[hp, j, odd], sem.at[0])
               for hp in range(heads // 2) for j, w in enumerate((wq_hbm, wk_hbm, wv_hbm)) for odd in range(2)]

    ZT = HS
    XS = ZT + FH
    WS = XS + HS // 2
    LF = WS + HF
    XL = LF + 13 * QF
    KF = XL + 2 * LANES

    def tok(q, j, base=0):
        r = base + (q * QS + j * LANES) // 2
        return slice(r, r + LANES // 2)

    def cols(q, j):
        return slice(q * QS + j * LANES, q * QS + (j + 1) * LANES)

    def left_at(p, r0, r1, c0, c1):
        r = LF + (p // 4) * QF
        return slice(r + r0, r + r1), slice((p % 4) * QS + c0, (p % 4) * QS + c1)

    def late_at(q, r0, r1, c0, c1):
        r = XL + (q // 2) * LANES
        return slice(r + r0, r + r1), slice((q % 2) * D + c0, (q % 2) * D + c1)

    def qkv_left_at(p, r0, r1):
        r = KF + (p // 16) * (LANES // 2)
        return slice(r + r0 // 2, r + r1 // 2), slice((p % 16) * LANES, (p % 16 + 1) * LANES)

    def ln_x(r, n, dep=None):
        xs = []
        for q in (r, HS + r):
            x = x_v[q:q + n, :].astype(F32)
            if dep is not None:
                x = jnp.concatenate([_after(x[:, :LANES], _tile(dep, n)), x[:, LANES:]], axis=1)
            xs.append(_layernorm(x))
            xn_v[q // 2:(q + n) // 2, :] = _pack(xs[-1])
            for t in range(q, q + n, LATE):
                if t % seg == seg - LATE:
                    g = t // seg // 4 * LATE
                    big_v[late_at(t // seg % 4, g, g + LATE, 0, D)] = pltpu.bitcast(xs[-1][t - q:t - q + LATE], U32)
        for i, p in enumerate(_RIGHT_SUMS):
            t = _strassen_right(p, lambda k, half: xs[half][:, k * KH:(k + 1) * KH])
            big_v[XS + r // 2:XS + (r + n) // 2, i * KH:(i + 1) * KH] = _pack(t)

    def ln_slices(j):
        for q in range(2):
            for r in range(q * QS + j * LANES, q * QS + (j + 1) * LANES, LN_ROWS):
                dep = yield
                ln_x(r, LN_ROWS, dep)

    def w_sums(which, a, b, dep=None):
        quad = [[_unpack(wint_v[which, (i * HF + a) // 2:(i * HF + b) // 2, k * KH:(k + 1) * KH]).astype(F32)
                 for k in range(2)] for i in range(2)]
        if dep is not None:
            dep = _tile(dep, b - a, KH)
            quad[0][0], quad[1][1] = _after(quad[0][0], dep), _after(quad[1][1], dep)
        left = _strassen_left(quad)
        r = WS + which * (HF // 2)
        for i, p in enumerate(_LEFT_SUMS):
            big_v[r + a // 2:r + b // 2, i * KH:(i + 1) * KH] = _pack(left[p])

    def w_sum_slices(which, a, b):
        for r in range(a, b, 16):
            dep = yield
            w_sums(which, r, r + 16, dep)

    def z_block(which, j, f, side, feed):
        tiles = [z_tile(which, j, q, f, side, feed) for q in range(2)]
        return [[jnp.concatenate([t[i][half] for t in tiles], axis=1) for half in range(2)] for i in range(2)]

    def z_tile(which, j, q, f, side, feed):
        def w(i, k):
            r = (i * HF + f) // 2
            return _unpack(wint_v[which, r:r + MB // 2, k * KH:min((k + 1) * KH, D)])

        def x(k, half):
            return _unpack(xn_v[tok(2 * half + q, j), k * KH:min((k + 1) * KH, D)])

        def left(p):
            if p not in _LEFT_SUMS:
                return w(p - 2, p - 2)
            i, r = _LEFT_SUMS.index(p), WS + (which * HF + f) // 2
            return _unpack(big_v[r:r + MB // 2, i * KH:(i + 1) * KH])

        def right(p):
            if p not in _RIGHT_SUMS:
                return x(p // 4, p // 4)
            i = _RIGHT_SUMS.index(p)
            return _unpack(big_v[tok(q, j, XS), i * KH:(i + 1) * KH])

        def dot(lhs, rhs):
            m = _dot_nt(lhs, rhs)
            side.feed(m, feed)
            return m

        return _strassen_combine(lambda p: dot(left(p), right(p)), jnp.add, jnp.subtract,
                                 lambda i, half, c: _gelu2(c + dot(w(i, 2), x(2, half))), plain_left_first=True)

    def finish_slices(j, sums, squares):
        ms, rs = [], []
        for half in range(2):
            m = jnp.sum(sums[half], axis=0, keepdims=True) * (1.0 / FH)
            v = jnp.maximum(jnp.sum(squares[half], axis=0, keepdims=True) * (1.0 / FH) - m * m, 0.0)
            r = lax.rsqrt(v + 4.0 * EPS)
            for q in range(2):
                ms.append(jnp.broadcast_to(m[:, q * LANES:(q + 1) * LANES], (8, LANES)))
                rs.append(jnp.broadcast_to(r[:, q * LANES:(q + 1) * LANES], (8, LANES)))
        for f in range(0, QF, 8):
            dep = yield
            mf = [_after(m, dep) for m in ms]
            a = [[(pltpu.bitcast(big_v[ZT + i * QF + f:ZT + i * QF + f + 8, cols(q, j)], F32) - mf[q]) * rs[q]
                  for q in range(4)] for i in range(4)]

            def emit(p, t):
                big_v[left_at(p, f, f + 8, j * LANES, (j + 1) * LANES)] = pltpu.bitcast(t, U32)

            yield from _left_factors(a, emit)

    def qkv_left_slices():
        for r in range(0, LANES, 16):
            a = [[pltpu.bitcast(big_v[late_at(q, r, r + 16, k * LANES, (k + 1) * LANES)], F32) for k in range(4)]
                 for q in range(4)]

            def emit(p, t):
                big_v[qkv_left_at(p, r, r + 16)] = _pack(t)

            yield from _left_factors(a, emit)

    def repack_slices():
        low = jnp.full((8, DH), 0xFFFF, U32)
        for hp in range(heads // 2):
            for j in range(3):
                for r in range(0, D // 2, PACK_ROWS):
                    dep = yield
                    m = _tile(_after(low, dep), PACK_ROWS)
                    even, odd = (stage_v[hp, j, k, r:r + PACK_ROWS, :] for k in range(2))
                    wqkv_v[2 * hp, r:r + PACK_ROWS, j * DH:(j + 1) * DH] = (even & m) | (odd << 16)
                    wqkv_v[2 * hp + 1, r:r + PACK_ROWS, j * DH:(j + 1) * DH] = (even >> 16) | (odd & ~m)

    def wout_sum_slices():
        for i, p in enumerate(_RIGHT_SUMS):
            for r in range(0, KY // 2, 16):
                dep = yield
                assert issued[0] > REST_WAIT_AT, "w_out has not been waited for yet"
                t = _strassen_right(p, lambda k, n: _unpack(
                    wout_v[k * KY // 2 + r:k * KY // 2 + r + 16, n * NY:(n + 1) * NY]).astype(F32))
                wsum_v[i, r:r + 16, :] = _pack(_after(t, _tile(dep, 32, NY)))

    start(x0_cps[0::2] + x0_cps[1::2] + w2a_cps + w2b_cps + x1_cps)
    late_v[...] = jnp.zeros(late_v.shape, F32)
    wait(x0_cps[0::2])
    ln_x(0, LANES)
    wait(x0_cps[1::2])
    ln_x(QS, LANES)
    wait(w2a_cps)
    w_sums(1, 0, MB)

    n_blocks = HF // MB
    products = 22
    ln_pieces = 2 * LANES // LN_ROWS
    finish_pieces = 7 * QF // 8

    side, finishes = _SideWork(), []
    for j in range(NB):
        sums, squares = [0.0, 0.0], [0.0, 0.0]
        for f in range(0, HF, MB):
            slots = (n_blocks - f // MB) * products
            if (j, f) == (0, MB):
                wait(w2b_cps)
                start(x2_cps + [bsp_cp, w1_cp, wsp_cp] + qkv_cps[:FIRST_COPIES])
                w_sums(1, MB, 2 * MB)
                side = _SideWork([w_sum_slices(1, 2 * MB, HF)], MB // 16, 0.7 * products * FEED_LN)
            if (j, f) == (0, 2 * MB):
                side.drain(partial)
                wait(x1_cps)
            if (j, f) == (1, MB):
                wait(x2_cps)
            if (j, f) in ((0, 2 * MB), (1, MB), (2, 0)):
                side = _SideWork([ln_slices(j + 1)], ln_pieces, LN_FILL[j] * slots * FEED_LN)
            if (j, f) == (NB - 1, 0):
                side = _SideWork([finishes.pop(0)], finish_pieces, FINISH_FILL * slots * FEED_FINISH)
            z = z_block(1, j, f, side, FEED_FINISH if j == NB - 1 else FEED_LN)
            for i in range(2):
                for half in range(2):
                    for q in range(2):
                        big_v[ZT + i * HF + f:ZT + i * HF + f + MB, cols(2 * half + q, j)] = pltpu.bitcast(
                            z[i][half][:, q * LANES:(q + 1) * LANES], U32)
                    partial = _vreg_sum(z[i][half])
                    sums[half] += partial
                    squares[half] += _vreg_sum(z[i][half] * z[i][half])
        side.drain(partial)
        finishes.append(finish_slices(j, sums, squares))
        if j == NB - 2:
            wait([bsp_cp, w1_cp])
            w_sums(0, 0, HF)

    side = _SideWork(finishes, len(finishes) * finish_pieces, FINISH_FILL * NB * n_blocks * products * FEED_FINISH)
    z1 = []
    for j in range(NB):
        z = [z_block(0, j, f, side, FEED_FINISH) for f in range(0, HF, MB)]
        z1.append([jnp.concatenate([blk[i][half] for i in range(2) for blk in z], axis=0) for half in range(2)])
    side.drain(z1[0][0])
    wsp_cp.wait()
    start(qkv_cps[FIRST_COPIES:] + late_cps)

    bias = bsp_v[...].astype(F32)
    issued, spatial_side = [0], [_SideWork([qkv_left_slices()], 6 * LANES // 16, 0.9 * QKV_WAIT_AT * 7 * FEED_PACK)]

    def count_products():
        if issued[0] == REST_WAIT_AT:
            wait(late_cps)
        if issued[0] == QKV_WAIT_AT:
            assert not spatial_side[0].gens
            pltpu.make_async_copy(stage_v, stage_v, sem.at[0]).wait()
            spatial_side[0] = _SideWork(
                [repack_slices(), wout_sum_slices()], (heads // 2) * 3 * (D // 2 // PACK_ROWS) + 5 * KY // 32,
                PACK_FILL * (7 * NB - QKV_WAIT_AT) * 7 * FEED_PACK)
        issued[0] += 1

    def spatial_product(p, rhs):
        m = _dot_nt(pltpu.bitcast(big_v[left_at(p, 0, QF, 0, QS)], F32), rhs)
        spatial_side[0].feed(m, FEED_PACK)
        return m

    for j in range(NB):
        c = _strassen_squared(spatial_product, lambda k, n: _unpack(big_v[tok(n, j), k * QS:(k + 1) * QS]),
                              before=count_products)
        for half in range(2):
            g = jnp.concatenate(
                [jnp.concatenate([c[i][2 * half + q] for i in range(4)], axis=0)
                 + bias[(2 * half + q) * NB + j:(2 * half + q) * NB + j + 1, :] for q in range(2)], axis=1)
            u = pltpu.bitcast((z1[j][half] * g).astype(BF16).T, U32)
            for q in range(2):
                u_v[tok(2 * half + q, j), :] = u[q * LANES // 2:(q + 1) * LANES // 2]
    spatial_side[0].drain(g)

    def late_qkv(a0):
        for j in range(3):
            c = _strassen_squared(
                lambda p, rhs: _dot(_unpack(big_v[qkv_left_at(p, 0, LANES)]), rhs),
                lambda k, n: _unpack(wqkv_v[a0 + n * (heads // 4), k * LANES // 2:(k + 1) * LANES // 2,
                                            j * DH:(j + 1) * DH]))
            for n in range(4):
                for pair in range(2):
                    stage_v[a0 // 2 + n * (heads // 8), j, a0 % 2, pair * LANES:(pair + 1) * LANES, :] = (
                        pltpu.pack_elementwise([c[2 * pair][n], c[2 * pair + 1][n]], packed_dtype=BF16))

    @pl.loop(0, QKV_LOOP)
    def _(i):
        for a0 in range(heads // 4 // QKV_LOOP):
            late_qkv(i * (heads // 4 // QKV_LOOP) + a0)


def _recurrence(out_hbm, x_v, mem_v, stage_v, wqkv_v, wo_v, wout_v, wsum_v, big_v, xn_v, u_v, late_v, o_v, out_v,
                sem_out, seg):
    heads, DH = wqkv_v.shape[0], wqkv_v.shape[2] // 3
    M, D = mem_v.shape
    n_groups = out_v.shape[0]
    early = seg - LATE
    KO = heads * DH // 4
    NO = 4 * LANES
    scale = DH ** -0.5
    row = lax.broadcasted_iota(jnp.int32, (M + seg, M + seg), 0)
    col = lax.broadcasted_iota(jnp.int32, (M + seg, M + seg), 1)
    ops = _segment_ops(heads)
    GL, XL, OF = 0, LANES, 2 * LANES

    def copy_out(at):
        pltpu.make_async_copy(out_v.at[at], out_hbm.at[at], sem_out).start()

    def factor_slices(g):
        for t in range(0, KO, FACTOR_COLS):
            a = [[late_v[k, :, c * KO + t:c * KO + t + FACTOR_COLS] for c in range(4)] for k in range(4)]

            def emit(p, f):
                c0 = (p % 2) * KO + t
                big_v[_rows(g, LATE, OF + p // 2 * LANES), c0:c0 + FACTOR_COLS] = pltpu.bitcast(f, U32)

            yield from _left_factors(a, emit)

    factor_pieces = 6 * KO // FACTOR_COLS

    def segment(g, k, mem, side, last):
        q0 = M if last else 0
        mask = ((row < M) | (row >= col))[q0:]
        h = jnp.concatenate([mem, _unpack(xn_v[_rows(4 * g + k, seg // 2), :]).astype(F32)], axis=0)
        qkv, probs, late, acc = {}, {}, [], None
        for op, a, *rest in ops:
            if op == "P":
                j = rest[0]
                c = slice(j * DH, (j + 1) * DH)
                batched = pltpu.unpack_elementwise(stage_v[a // 2, j, a % 2, _rows(g, LATE, k // 2 * LANES), :],
                                                   index=k % 2, packed_dtype=BF16, unpacked_dtype=F32)
                qkv[a, j] = (
                    jnp.concatenate([_dot(h[:M + early, :2 * KH], _unpack(wqkv_v[a, :KH, c])), batched], axis=0)
                    + _dot(h[:, 2 * KH:], _unpack(wqkv_v[a, KH:, c])))
                side.feed(qkv[a, j], 2 if j == 0 else 0)
            elif op == "S":
                scores = jnp.where(mask, _dot_nt(qkv.pop((a, 0))[q0:], qkv.pop((a, 1))) * scale, -1e9)
                e = jnp.exp(scores - jnp.max(scores, axis=-1, keepdims=True))
                probs[a] = e, _recip(jnp.sum(e, axis=-1, keepdims=True))
            elif op == "V":
                e, inv = probs.pop(a)
                o = _dot(e, qkv.pop((a, 2))) * inv
                o_v[q0:, a * DH:(a + 1) * DH] = o
                late.append(o[-LATE:])
                if a == heads - 1:
                    assert not side.gens, "the previous group's outputs are still being read"
                    late_v[k] = jnp.concatenate(late, axis=1)
                    if last:
                        side = _SideWork([factor_slices(g)], factor_pieces, 12)
            else:
                b = rest[0]
                w = slice(a * DH // 2, b * DH // 2)
                part = [_dot(o_v[q0:M + early, a * DH:b * DH], _unpack(wo_v[w, n:n + LANES]))
                        for n in range(0, NO, LANES)] + [_dot(o_v[q0:, a * DH:b * DH], _unpack(wo_v[w, NO:]))]
                acc = part if acc is None else [t + p for t, p in zip(acc, part)]
        for p in part[:4]:
            side.feed(p, 3)
        side.drain(part[3])
        out = jnp.concatenate(acc[:-1] + [acc[-1][:-LATE]], axis=1)
        return out[:M], out[M - q0:], acc[-1][-LATE:]

    def segment_pair(g, k, mem, followed, side, last=False):
        u = _unpack(u_v[_rows(2 * g + k // 2, seg), :])
        left = _strassen_left([[u[i * seg:(i + 1) * seg, c * KY:(c + 1) * KY].astype(F32) for c in range(2)]
                               for i in range(2)])

        def product(p):
            if p in _RIGHT_SUMS:
                return _dot(left[p], _unpack(wsum_v[_RIGHT_SUMS.index(p)]))
            c = p // 4
            return _dot(left[p], _unpack(wout_v[c * KY // 2:(c + 1) * KY // 2, c * NY:(c + 1) * NY]))

        def gate(done):
            c = _strassen_combine(lambda p: done[p] if p in done else product(p), jnp.add, jnp.subtract)
            return _silu_of_half(jnp.concatenate(
                [jnp.concatenate([jnp.concatenate(r, axis=1) for r in c], axis=0)
                 + _dot(u[:, 2 * KY:], _unpack(wout_v[KY:, :2 * NY])),
                 _dot(u, _unpack(wout_v[:, 2 * NY:]))], axis=1))

        mem, *first = segment(g, k, mem, side, False)
        done = {p: product(p) for p in EARLY_PRODUCTS}
        gates = None if followed else gate(done)
        mem, *second = segment(g, k + 1, mem, side, last)
        gates = gate(done) if followed else gates
        for i, (attn, late_attn) in enumerate((first, second)):
            x = x_v[_rows(4 * g + k + i, seg), :].astype(F32)
            gt = gates[i * seg:(i + 1) * seg]
            out_v[g, k + i, :early, :] = (x[:early] + attn * gt[:early]).astype(out_v.dtype)
            out_v[g, k + i, early:, NO:] = (x[early:, NO:] + late_attn * gt[early:, NO:]).astype(out_v.dtype)
            for base, t in ((GL, gt), (XL, x)):
                big_v[_rows(g, LATE, base), (k + i) * NO:(k + i + 1) * NO] = pltpu.bitcast(t[early:, :NO], U32)
        return mem

    def group(g, mem, last=False):
        previous = g - 1 if last else jnp.maximum(g - 1, 0)
        side = _SideWork([factor_slices(previous)], factor_pieces, FACTOR_FILL * 2 * heads)
        mem = segment_pair(g, 0, mem, True, side)
        mem = segment_pair(g, 2, mem, False, side, last)
        if not last:
            copy_out((g, slice(None), slice(0, early)))
        return mem

    mem = lax.fori_loop(0, n_groups - 1, group, mem_v[...].astype(F32))
    group(n_groups - 1, mem, last=True)

    ready = [[], [], [(n_groups - 1, slice(None), slice(0, early)),
                  (slice(None), slice(None), slice(early, seg), slice(NO, D))]]

    def issue_copies():
        for at in ready.pop(0):
            copy_out(at)
        ready.append([])

    def late_output(k, n, c):
        t = slice(n * LANES, (n + 1) * LANES)
        gt, x = (pltpu.bitcast(big_v[base:base + LANES, k * NO + t.start:k * NO + t.stop], F32) for base in (GL, XL))
        out_v[:, k, early:, t] = (x + c * gt).reshape(n_groups, LATE, LANES).astype(out_v.dtype)
        ready[-1].append((slice(None), k, slice(early, seg), t))

    def late_product(p, rhs):
        issue_copies()
        return _dot(pltpu.bitcast(big_v[_rows(p // 2, LANES, OF), (p % 2) * KO:(p % 2 + 1) * KO], F32), rhs)

    _strassen_squared(
        late_product, lambda k, n: _unpack(wo_v[k * KO // 2:(k + 1) * KO // 2, n * LANES:(n + 1) * LANES]), late_output,
        dtype=BF16)
    for _ in ready:
        issue_copies()
    pltpu.make_async_copy(out_v, out_hbm, sem_out).wait()


def _kernel(x_hbm, mem_hbm, wq_hbm, wk_hbm, wv_hbm, wo_hbm, wint_hbm, wsp_hbm, bsp_hbm, wout_hbm, out_hbm,
            x_v, mem_v, stage_v, wqkv_v, wo_v, wint_v, big_v, bsp_v, wout_v, wsum_v, xn_v, u_v, late_v,
            o_v, out_v, sem, sem_out, *, seg):
    _gating_branch(x_hbm, mem_hbm, wq_hbm, wk_hbm, wv_hbm, wo_hbm, wint_hbm, wsp_hbm, bsp_hbm, wout_hbm,
                   x_v, mem_v, stage_v, wqkv_v, wo_v, wint_v, big_v, bsp_v, wout_v, wsum_v, xn_v, u_v, late_v,
                   sem, seg)
    _recurrence(out_hbm, x_v, mem_v, stage_v, wqkv_v, wo_v, wout_v, wsum_v, big_v, xn_v, u_v, late_v, o_v, out_v,
                sem_out, seg)


@functools.partial(jax.jit, static_argnames=("A_seg_len",))
def pallas_recurrent_scan__memory_aug_recurrent_mem_tr__mixer_gmlp__prompt_kernel(
    A_x, A_mem0, A_Wq, A_Wk, A_Wv, A_Wo, A_seg_len, B_x, B_w_in, B_w_sp, B_b_sp, B_w_out,
):
    del B_x
    B, S, D = A_x.shape
    M = A_mem0.shape[1]
    _, H, DH = A_Wq.shape
    FH = B_w_in.shape[1] // 2
    seg = int(A_seg_len)
    assert B == 1 and DH == LANES and S == 16 * LANES and H == O_GROUPS[-1]
    assert D == 2 * KH + LANES == 2 * NY + LANES and FH == 6 * MB and 2 * KY < FH and S // seg * LATE == 4 * LANES
    big_rows = S // 2 + FH + S // 4 + FH // 2 + 13 * (FH // 4) + 4 * LANES
    groups = (S // seg // 4, 4, seg, D)
    out = pl.pallas_call(
        functools.partial(_kernel, seg=seg),
        out_shape=jax.ShapeDtypeStruct(groups, A_x.dtype),
        in_specs=[pl.BlockSpec(memory_space=pl.ANY)] * 10,
        out_specs=pl.BlockSpec(memory_space=pl.ANY),
        scratch_shapes=[
            pltpu.VMEM((S, D), BF16),
            pltpu.VMEM((M, D), BF16),
            pltpu.VMEM((H // 2, 3, 2, D // 2, DH), U32),
            pltpu.VMEM((H, D // 2, 3 * DH), U32),
            pltpu.VMEM((H * DH // 2, D), U32),
            pltpu.VMEM((2, FH // 2, D), U32),
            pltpu.VMEM((big_rows, S), U32),
            pltpu.VMEM((S // LANES, LANES), BF16),
            pltpu.VMEM((FH // 2, D), U32),
            pltpu.VMEM((5, KY // 2, NY), U32),
            pltpu.VMEM((S // 2, D), U32),
            pltpu.VMEM((S // 2, FH), U32),
            pltpu.VMEM((4, LATE, H * DH), F32),
            pltpu.VMEM((M + seg, H * DH), F32),
            pltpu.VMEM(groups, BF16),
            pltpu.SemaphoreType.DMA((24,)),
            pltpu.SemaphoreType.DMA(()),
        ],
        compiler_params=pltpu.CompilerParams(vmem_limit_bytes=120 * 1024 * 1024, disable_bounds_checks=True),
    )(
        A_x.reshape(S, D), A_mem0.reshape(M, D),
        *[w.reshape(D // 2, 2, H // 2, 2, DH) for w in (A_Wq, A_Wk, A_Wv)],
        A_Wo.reshape(H * DH, D), B_w_in.T, B_w_sp, B_b_sp.reshape(S // LANES, LANES), B_w_out,
    )
    return out.reshape(B, S, D)
```

```python
import functools

import jax
import jax.numpy as jnp
from jax import lax
from jax.experimental import pallas as pl
from jax.experimental.pallas import tpu as pltpu

F32 = jnp.float32
BF16 = jnp.bfloat16
U32 = jnp.uint32
EPS = 1e-5
NT = (((1,), (1,)), ((), ()))

LANES = 128
KH = 256
KY, NY = 384, 256
MB = 144
LATE = 8

LN_ROWS = 16
PACK_ROWS = 16
FEED_LN, FEED_FINISH, FEED_PACK = 2, 4, 13
LN_FILL, FINISH_FILL, PACK_FILL = (0.35, 0.6, 0.8), 0.9, 0.98
FIRST_COPIES = 56
QKV_WAIT_AT, REST_WAIT_AT = 18, 26
S_LAG, V_LAG = 2, 5
O_GROUPS = (0, 2, 5, 11, 32)
EARLY_PRODUCTS = (1, 3, 4, 2)
FACTOR_COLS, FACTOR_FILL = 512, 0.85
QKV_LOOP = 2


def _layernorm(x):
    m = jnp.mean(x, axis=-1, keepdims=True)
    d = x - m
    v = jnp.mean(d * d, axis=-1, keepdims=True)
    return d * lax.rsqrt(v + EPS)


def _gelu2(x):
    c = 0.7978845608028654
    return x + x * jnp.tanh(x * (c + (c * 0.044715) * (x * x)))


def _silu_of_half(y2):
    hy = 0.25 * y2
    return hy + hy * jnp.tanh(hy)


def _recip(l):
    r = pl.reciprocal(l, approx=True)
    return r + r * (1.0 - l * r)


def _pack(w):
    return pltpu.bitcast(w.astype(BF16), U32)


def _unpack(w32):
    return pltpu.bitcast(w32, BF16)


def _dot(a, b):
    return jnp.dot(a, b, preferred_element_type=F32)


def _dot_nt(a, b):
    return lax.dot_general(a, b, NT, preferred_element_type=F32)


def _vreg_sum(x):
    return jnp.sum(x.reshape(x.shape[0] // 8, 8, x.shape[1]), axis=0)


def _rows(i, n, base=0):
    start = base + i * n
    return pl.ds(start if isinstance(i, int) else pl.multiple_of(start, n), n)


def _tile(v, rows, cols=LANES):
    return jnp.concatenate([jnp.concatenate([v] * (rows // 8), axis=0)] * (cols // LANES), axis=1)


def _after(val, dep):
    return jnp.where(dep * dep < 0.0, pltpu.bitcast(dep, val.dtype), val)


class _SideWork:
    def __init__(self, gens=(), pieces=0, slots=1):
        self.gens, self.rate, self.credit = list(gens), pieces / slots, 0.0
        for g in self.gens:
            next(g)

    def feed(self, m, k=1):
        for t in range(k):
            self.credit += self.rate
            while self.gens and self.credit >= 1.0:
                self.credit -= 1.0
                r = t * (m.shape[0] // 8) // k * 8
                try:
                    self.gens[0].send(m[r:r + 8, :LANES])
                except StopIteration:
                    self.gens.pop(0)

    def drain(self, m):
        while self.gens:
            self.credit += 1.0
            self.feed(m)


def _strassen_left(a):
    return (a[0][0] + a[1][1], a[1][0] + a[1][1], a[0][0], a[1][1],
            a[0][0] + a[0][1], a[1][0] - a[0][0], a[0][1] - a[1][1])


_RIGHT_TERMS = (((0, 0), (1, 1), 1), ((0, 0), None, 0), ((0, 1), (1, 1), -1), ((1, 0), (0, 0), -1),
                ((1, 1), None, 0), ((0, 0), (0, 1), 1), ((1, 0), (1, 1), 1))
_LEFT_SUMS = (0, 1, 4, 5, 6)
_RIGHT_SUMS = (0, 2, 3, 5, 6)


def _strassen_right(p, b):
    first, second, sign = _RIGHT_TERMS[p]
    if second is None:
        return b(*first)
    return b(*first) + b(*second) if sign > 0 else b(*first) - b(*second)


def _strassen_combine(product, done=lambda i, n, c: c, plain_left_first=False):
    if plain_left_first:
        m3, m4, m5 = product(2), product(3), product(4)
        c12 = done(0, 1, m3 + m5)
        m2 = product(1)
        c21 = done(1, 0, m2 + m4)
    else:
        m2, m4 = product(1), product(3)
        c21 = done(1, 0, m2 + m4)
        m5, m3 = product(4), product(2)
        c12 = done(0, 1, m3 + m5)
    d1, d2 = m4 - m5, m3 - m2
    m1 = product(0)
    d1, d2 = d1 + m1, d2 + m1
    c11 = done(0, 0, d1 + product(6))
    c22 = done(1, 1, d2 + product(5))
    return (c11, c12), (c21, c22)


def _left_factors(a, emit):
    outer = [[_strassen_left([[a[2 * i + i2][2 * k + k2] for k in range(2)] for i in range(2)])
              for k2 in range(2)] for i2 in range(2)]
    for p in range(7):
        quad = [[outer[i2][k2][p] for k2 in range(2)] for i2 in range(2)]
        if p:
            dep = _tile((yield), *quad[0][0].shape)
            quad[0][0], quad[1][1] = _after(quad[0][0], dep), _after(quad[1][1], dep)
        for p2, t in enumerate(_strassen_left(quad)):
            emit(7 * p + p2, t)


def _strassen_squared(product, block, done, before=lambda: None, dtype=F32):
    def quadrantwise(op):
        return lambda a, b: [[op(a[i][n], b[i][n]) for n in range(2)] for i in range(2)]

    add, sub = quadrantwise(jnp.add), quadrantwise(jnp.subtract)

    def outer(p, i=None, n=None, partial=None):
        def finish(i2, n2, t):
            if partial:
                done(2 * i + i2, 2 * n + n2, partial[i2][n2] + t)
            return t

        before()
        b = [[_strassen_right(p, lambda k, m: block(2 * k + k2, 2 * m + n2).astype(F32))
              for n2 in range(2)] for k2 in range(2)]
        return _strassen_combine(
            lambda p2: product(7 * p + p2, _strassen_right(p2, lambda k, m: b[k][m]).astype(dtype)), finish)

    m2 = outer(1)
    m4 = outer(3, 1, 0, m2)
    m5 = outer(4)
    m3 = outer(2, 0, 1, m5)
    d1, d2 = sub(m4, m5), sub(m3, m2)
    m1 = outer(0)
    outer(6, 0, 0, add(d1, m1))
    outer(5, 1, 1, add(d2, m1))


def _segment_ops(heads):
    groups = [("O", a, b) for a, b in zip(O_GROUPS[:-1], O_GROUPS[1:])]
    ops = []
    for t in range(heads):
        ops += [("P", t, j) for j in range(3)]
        ops += [(op, t - lag) for op, lag in (("V", V_LAG), ("S", S_LAG)) if t >= lag]
        if t == groups[0][2] + V_LAG:
            ops.append(groups[0])
    scores = [("S", a) for a in range(heads - S_LAG, heads)]
    values = [("V", a) for a in range(heads - V_LAG, heads)]
    return ops + [groups[1]] + scores + values[:1] + [groups[2]] + values[1:] + groups[3:]


def _gating_branch(x_hbm, mem_hbm, wq_hbm, wk_hbm, wv_hbm, wo_hbm, wint_hbm, wsp_hbm, bsp_hbm, wout_hbm,
                   x_v, mem_v, stage_v, wqkv_v, wo_v, wint_v, big_v, bsp_v, wout_v, wsum_v, xn_v, u_v, late_v,
                   sem, seg):
    S, D = x_v.shape
    heads, DH = wqkv_v.shape[0], wqkv_v.shape[2] // 3
    FH = u_v.shape[1]
    HS, QS = S // 2, S // 4
    HF, QF = FH // 2, FH // 4
    NB = QS // LANES
    n_sem = [0]

    def copy(src, dst):
        n_sem[0] += 1
        return pltpu.make_async_copy(src, dst, sem.at[n_sem[0]])

    def start(cps):
        for cp in cps:
            cp.start()

    def wait(cps):
        for cp in cps:
            cp.wait()

    def x_copies(a, b):
        rs = [slice(q * QS + a * LANES, q * QS + b * LANES) for q in range(4)]
        return [copy(x_hbm.at[r], x_v.at[r]) for r in rs]

    x0_cps, x1_cps, x2_cps = x_copies(0, 1), x_copies(1, 2), x_copies(2, NB)
    w1_cp = copy(wint_hbm.bitcast(U32).at[:HF], wint_v.at[0])

    def w2_copies(a, b):
        rs = [slice((i * HF + a) // 2, (i * HF + b) // 2) for i in range(2)]
        return [copy(wint_hbm.bitcast(U32).at[HF + r.start:HF + r.stop], wint_v.at[1, r]) for r in rs]

    w2a_cps, w2b_cps = w2_copies(0, MB), w2_copies(MB, HF)
    bsp_cp = copy(bsp_hbm, bsp_v)
    wsp_cp = copy(wsp_hbm.bitcast(U32), big_v.at[:HS])
    late_cps = [copy(mem_hbm, mem_v), copy(wout_hbm.bitcast(U32), wout_v), copy(wo_hbm.bitcast(U32), wo_v)]
    qkv_cps = [pltpu.make_async_copy(w.bitcast(U32).at[:, odd, hp, 0], stage_v.at[hp, j, odd], sem.at[0])
               for hp in range(heads // 2) for j, w in enumerate((wq_hbm, wk_hbm, wv_hbm)) for odd in range(2)]

    ZT = HS
    XS = ZT + FH
    WS = XS + HS // 2
    LF = WS + HF
    XL = LF + 13 * QF
    KF = XL + 2 * LANES

    def tok(q, j, base=0):
        r = base + (q * QS + j * LANES) // 2
        return slice(r, r + LANES // 2)

    def cols(q, j):
        return slice(q * QS + j * LANES, q * QS + (j + 1) * LANES)

    def left_at(p, r0, r1, c0, c1):
        r = LF + (p // 4) * QF
        return slice(r + r0, r + r1), slice((p % 4) * QS + c0, (p % 4) * QS + c1)

    def late_at(q, r0, r1, c0, c1):
        r = XL + (q // 2) * LANES
        return slice(r + r0, r + r1), slice((q % 2) * D + c0, (q % 2) * D + c1)

    def qkv_left_at(p, r0, r1):
        r = KF + (p // 16) * (LANES // 2)
        return slice(r + r0 // 2, r + r1 // 2), slice((p % 16) * LANES, (p % 16 + 1) * LANES)

    def ln_x(r, n, dep=None):
        xs = []
        for q in (r, HS + r):
            x = x_v[q:q + n, :].astype(F32)
            if dep is not None:
                x = jnp.concatenate([_after(x[:, :LANES], _tile(dep, n)), x[:, LANES:]], axis=1)
            xs.append(_layernorm(x))
            xn_v[q // 2:(q + n) // 2, :] = _pack(xs[-1])
            for t in range(q, q + n, LATE):
                if t % seg == seg - LATE:
                    g = t // seg // 4 * LATE
                    big_v[late_at(t // seg % 4, g, g + LATE, 0, D)] = pltpu.bitcast(xs[-1][t - q:t - q + LATE], U32)
        for i, p in enumerate(_RIGHT_SUMS):
            t = _strassen_right(p, lambda k, half: xs[half][:, k * KH:(k + 1) * KH])
            big_v[XS + r // 2:XS + (r + n) // 2, i * KH:(i + 1) * KH] = _pack(t)

    def ln_slices(j):
        for q in range(2):
            for r in range(q * QS + j * LANES, q * QS + (j + 1) * LANES, LN_ROWS):
                dep = yield
                ln_x(r, LN_ROWS, dep)

    def w_sums(which, a, b, dep=None):
        quad = [[_unpack(wint_v[which, (i * HF + a) // 2:(i * HF + b) // 2, k * KH:(k + 1) * KH]).astype(F32)
                 for k in range(2)] for i in range(2)]
        if dep is not None:
            dep = _tile(dep, b - a, KH)
            quad[0][0], quad[1][1] = _after(quad[0][0], dep), _after(quad[1][1], dep)
        left = _strassen_left(quad)
        r = WS + which * (HF // 2)
        for i, p in enumerate(_LEFT_SUMS):
            big_v[r + a // 2:r + b // 2, i * KH:(i + 1) * KH] = _pack(left[p])

    def w_sum_slices(which, a, b):
        for r in range(a, b, 16):
            dep = yield
            w_sums(which, r, r + 16, dep)

    def z_block(which, j, f, side, feed):
        tiles = [z_tile(which, j, q, f, side, feed) for q in range(2)]
        return [[jnp.concatenate([t[i][half] for t in tiles], axis=1) for half in range(2)] for i in range(2)]

    def z_tile(which, j, q, f, side, feed):
        def w(i, k):
            r = (i * HF + f) // 2
            return _unpack(wint_v[which, r:r + MB // 2, k * KH:min((k + 1) * KH, D)])

        def x(k, half):
            return _unpack(xn_v[tok(2 * half + q, j), k * KH:min((k + 1) * KH, D)])

        def left(p):
            if p not in _LEFT_SUMS:
                return w(p - 2, p - 2)
            i, r = _LEFT_SUMS.index(p), WS + (which * HF + f) // 2
            return _unpack(big_v[r:r + MB // 2, i * KH:(i + 1) * KH])

        def right(p):
            if p not in _RIGHT_SUMS:
                return x(p // 4, p // 4)
            i = _RIGHT_SUMS.index(p)
            return _unpack(big_v[tok(q, j, XS), i * KH:(i + 1) * KH])

        def dot(lhs, rhs):
            m = _dot_nt(lhs, rhs)
            side.feed(m, feed)
            return m

        return _strassen_combine(lambda p: dot(left(p), right(p)),
                                 lambda i, half, c: _gelu2(c + dot(w(i, 2), x(2, half))), plain_left_first=True)

    def finish_slices(j, sums, squares):
        ms, rs = [], []
        for half in range(2):
            m = jnp.sum(sums[half], axis=0, keepdims=True) * (1.0 / FH)
            v = jnp.maximum(jnp.sum(squares[half], axis=0, keepdims=True) * (1.0 / FH) - m * m, 0.0)
            r = lax.rsqrt(v + 4.0 * EPS)
            for q in range(2):
                ms.append(jnp.broadcast_to(m[:, q * LANES:(q + 1) * LANES], (8, LANES)))
                rs.append(jnp.broadcast_to(r[:, q * LANES:(q + 1) * LANES], (8, LANES)))
        for f in range(0, QF, 8):
            dep = yield
            mf = [_after(m, dep) for m in ms]
            a = [[(pltpu.bitcast(big_v[ZT + i * QF + f:ZT + i * QF + f + 8, cols(q, j)], F32) - mf[q]) * rs[q]
                  for q in range(4)] for i in range(4)]

            def emit(p, t):
                big_v[left_at(p, f, f + 8, j * LANES, (j + 1) * LANES)] = pltpu.bitcast(t, U32)

            yield from _left_factors(a, emit)

    def qkv_left_slices():
        for r in range(0, LANES, 16):
            a = [[pltpu.bitcast(big_v[late_at(q, r, r + 16, k * LANES, (k + 1) * LANES)], F32) for k in range(4)]
                 for q in range(4)]

            def emit(p, t):
                big_v[qkv_left_at(p, r, r + 16)] = _pack(t)

            yield from _left_factors(a, emit)

    def repack_slices():
        low = jnp.full((8, DH), 0xFFFF, U32)
        for hp in range(heads // 2):
            for j in range(3):
                for r in range(0, D // 2, PACK_ROWS):
                    dep = yield
                    m = _tile(_after(low, dep), PACK_ROWS)
                    even, odd = (stage_v[hp, j, k, r:r + PACK_ROWS, :] for k in range(2))
                    wqkv_v[2 * hp, r:r + PACK_ROWS, j * DH:(j + 1) * DH] = (even & m) | (odd << 16)
                    wqkv_v[2 * hp + 1, r:r + PACK_ROWS, j * DH:(j + 1) * DH] = (even >> 16) | (odd & ~m)

    def wout_sum_slices():
        for i, p in enumerate(_RIGHT_SUMS):
            for r in range(0, KY // 2, 16):
                dep = yield
                assert issued[0] > REST_WAIT_AT, "w_out has not been waited for yet"
                t = _strassen_right(p, lambda k, n: _unpack(
                    wout_v[k * KY // 2 + r:k * KY // 2 + r + 16, n * NY:(n + 1) * NY]).astype(F32))
                wsum_v[i, r:r + 16, :] = _pack(_after(t, _tile(dep, 32, NY)))

    start(x0_cps[0::2] + x0_cps[1::2] + w2a_cps + w2b_cps + x1_cps)
    late_v[...] = jnp.zeros(late_v.shape, F32)
    wait(x0_cps[0::2])
    ln_x(0, LANES)
    wait(x0_cps[1::2])
    ln_x(QS, LANES)
    wait(w2a_cps)
    w_sums(1, 0, MB)

    n_blocks = HF // MB
    products = 22
    ln_pieces = 2 * LANES // LN_ROWS
    finish_pieces = 7 * QF // 8

    side, finishes = _SideWork(), []
    for j in range(NB):
        sums, squares = [0.0, 0.0], [0.0, 0.0]
        for f in range(0, HF, MB):
            slots = (n_blocks - f // MB) * products
            if (j, f) == (0, MB):
                wait(w2b_cps)
                start(x2_cps + [bsp_cp, w1_cp, wsp_cp] + qkv_cps[:FIRST_COPIES])
                w_sums(1, MB, 2 * MB)
                side = _SideWork([w_sum_slices(1, 2 * MB, HF)], MB // 16, 0.7 * products * FEED_LN)
            if (j, f) == (0, 2 * MB):
                side.drain(partial)
                wait(x1_cps)
            if (j, f) == (1, MB):
                wait(x2_cps)
            if (j, f) in ((0, 2 * MB), (1, MB), (2, 0)):
                side = _SideWork([ln_slices(j + 1)], ln_pieces, LN_FILL[j] * slots * FEED_LN)
            if (j, f) == (NB - 1, 0):
                side = _SideWork([finishes.pop(0)], finish_pieces, FINISH_FILL * slots * FEED_FINISH)
            z = z_block(1, j, f, side, FEED_FINISH if j == NB - 1 else FEED_LN)
            for i in range(2):
                for half in range(2):
                    for q in range(2):
                        big_v[ZT + i * HF + f:ZT + i * HF + f + MB, cols(2 * half + q, j)] = pltpu.bitcast(
                            z[i][half][:, q * LANES:(q + 1) * LANES], U32)
                    partial = _vreg_sum(z[i][half])
                    sums[half] += partial
                    squares[half] += _vreg_sum(z[i][half] * z[i][half])
        side.drain(partial)
        finishes.append(finish_slices(j, sums, squares))
        if j == NB - 2:
            wait([bsp_cp, w1_cp])
            w_sums(0, 0, HF)

    side = _SideWork(finishes, len(finishes) * finish_pieces, FINISH_FILL * NB * n_blocks * products * FEED_FINISH)
    z1 = []
    for j in range(NB):
        z = [z_block(0, j, f, side, FEED_FINISH) for f in range(0, HF, MB)]
        z1.append([jnp.concatenate([blk[i][half] for i in range(2) for blk in z], axis=0) for half in range(2)])
    side.drain(z1[0][0])
    wsp_cp.wait()
    start(qkv_cps[FIRST_COPIES:] + late_cps)

    bias = bsp_v[...].astype(F32)
    issued, spatial_side = [0], [_SideWork([qkv_left_slices()], 6 * LANES // 16, 0.9 * QKV_WAIT_AT * 7 * FEED_PACK)]

    def count_products():
        if issued[0] == REST_WAIT_AT:
            wait(late_cps)
        if issued[0] == QKV_WAIT_AT:
            assert not spatial_side[0].gens
            pltpu.make_async_copy(stage_v, stage_v, sem.at[0]).wait()
            spatial_side[0] = _SideWork(
                [repack_slices(), wout_sum_slices()], (heads // 2) * 3 * (D // 2 // PACK_ROWS) + 5 * KY // 32,
                PACK_FILL * (7 * NB - QKV_WAIT_AT) * 7 * FEED_PACK)
        issued[0] += 1

    def spatial_product(p, rhs):
        m = _dot_nt(pltpu.bitcast(big_v[left_at(p, 0, QF, 0, QS)], F32), rhs)
        spatial_side[0].feed(m, FEED_PACK)
        return m

    for j in range(NB):
        gated = {}

        def gate_block(i, n, g):
            half = n // 2
            gated[i, n] = (z1[j][half][i * QF:(i + 1) * QF, n % 2 * LANES:(n % 2 + 1) * LANES]
                           * (g + bias[n * NB + j:n * NB + j + 1, :]))
            if all((r, 2 * half + q) in gated for r in range(4) for q in range(2)):
                u = jnp.concatenate([jnp.concatenate([gated[r, 2 * half + q] for r in range(4)], axis=0)
                                     for q in range(2)], axis=1)
                u = pltpu.bitcast(u.astype(BF16).T, U32)
                for q in range(2):
                    u_v[tok(2 * half + q, j), :] = u[q * LANES // 2:(q + 1) * LANES // 2]

        _strassen_squared(spatial_product, lambda k, n: _unpack(big_v[tok(n, j), k * QS:(k + 1) * QS]),
                          gate_block, count_products)
    spatial_side[0].drain(gated[3, 3])

    def late_qkv(a0):
        for j in range(3):
            c = {}

            def done(i, n, t):
                c[i, n] = pltpu.bitcast(t.astype(BF16).astype(F32), U32)

            _strassen_squared(
                lambda p, rhs: _dot(_unpack(big_v[qkv_left_at(p, 0, LANES)]), rhs),
                lambda k, n: _unpack(wqkv_v[a0 + n * (heads // 4), k * LANES // 2:(k + 1) * LANES // 2,
                                            j * DH:(j + 1) * DH]), done)
            for n in range(4):
                for pair in range(2):
                    stage_v[a0 // 2 + n * (heads // 8), j, a0 % 2, pair * LANES:(pair + 1) * LANES, :] = (
                        (c[2 * pair, n] >> 16) | c[2 * pair + 1, n])

    @pl.loop(0, QKV_LOOP)
    def _(i):
        for a0 in range(heads // 4 // QKV_LOOP):
            late_qkv(i * (heads // 4 // QKV_LOOP) + a0)


def _recurrence(out_hbm, x_v, mem_v, stage_v, wqkv_v, wo_v, wout_v, wsum_v, big_v, xn_v, u_v, late_v, o_v, out_v,
                sem_out, seg):
    heads, DH = wqkv_v.shape[0], wqkv_v.shape[2] // 3
    M, D = mem_v.shape
    n_groups = out_v.shape[0]
    early = seg - LATE
    KO = heads * DH // 4
    NO = 4 * LANES
    scale = DH ** -0.5
    row = lax.broadcasted_iota(jnp.int32, (M + seg, M + seg), 0)
    col = lax.broadcasted_iota(jnp.int32, (M + seg, M + seg), 1)
    ops = _segment_ops(heads)
    GL, XL, OF = 0, LANES, 2 * LANES

    def copy_out(at):
        pltpu.make_async_copy(out_v.at[at], out_hbm.at[at], sem_out).start()

    def factor_slices(g):
        for t in range(0, KO, FACTOR_COLS):
            a = [[late_v[k, :, c * KO + t:c * KO + t + FACTOR_COLS] for c in range(4)] for k in range(4)]

            def emit(p, f):
                c0 = (p % 2) * KO + t
                big_v[_rows(g, LATE, OF + p // 2 * LANES), c0:c0 + FACTOR_COLS] = pltpu.bitcast(f, U32)

            yield from _left_factors(a, emit)

    factor_pieces = 6 * KO // FACTOR_COLS

    def segment(g, k, mem, side, last):
        q0 = M if last else 0
        mask = ((row < M) | (row >= col))[q0:]
        h = jnp.concatenate([mem, _unpack(xn_v[_rows(4 * g + k, seg // 2), :]).astype(F32)], axis=0)
        qkv, probs, late, acc = {}, {}, [], None
        for op, a, *rest in ops:
            if op == "P":
                j = rest[0]
                c = slice(j * DH, (j + 1) * DH)
                words = stage_v[a // 2, j, a % 2, _rows(g, LATE, k // 2 * LANES), :]
                batched = pltpu.bitcast(words & jnp.uint32(0xFFFF0000) if k % 2 else words << 16, F32)
                qkv[a, j] = (
                    jnp.concatenate([_dot(h[:M + early, :2 * KH], _unpack(wqkv_v[a, :KH, c])), batched], axis=0)
                    + _dot(h[:, 2 * KH:], _unpack(wqkv_v[a, KH:, c])))
                side.feed(qkv[a, j], 2 if j == 0 else 0)
            elif op == "S":
                scores = jnp.where(mask, _dot_nt(qkv.pop((a, 0))[q0:], qkv.pop((a, 1))) * scale, -1e9)
                e = jnp.exp(scores - jnp.max(scores, axis=-1, keepdims=True))
                probs[a] = e, _recip(jnp.sum(e, axis=-1, keepdims=True))
            elif op == "V":
                e, inv = probs.pop(a)
                o = _dot(e, qkv.pop((a, 2))) * inv
                o_v[q0:, a * DH:(a + 1) * DH] = o
                late.append(o[-LATE:])
                if a == heads - 1:
                    assert not side.gens, "the previous group's outputs are still being read"
                    late_v[k] = jnp.concatenate(late, axis=1)
                    if last:
                        side = _SideWork([factor_slices(g)], factor_pieces, 12)
            else:
                b = rest[0]
                w = slice(a * DH // 2, b * DH // 2)
                part = [_dot(o_v[q0:M + early, a * DH:b * DH], _unpack(wo_v[w, n:n + LANES]))
                        for n in range(0, NO, LANES)] + [_dot(o_v[q0:, a * DH:b * DH], _unpack(wo_v[w, NO:]))]
                acc = part if acc is None else [t + p for t, p in zip(acc, part)]
        for p in part[:4]:
            side.feed(p, 3)
        side.drain(part[3])
        out = jnp.concatenate(acc[:-1] + [acc[-1][:-LATE]], axis=1)
        return out[:M], out[M - q0:], acc[-1][-LATE:]

    def segment_pair(g, k, mem, followed, side, last=False):
        u = _unpack(u_v[_rows(2 * g + k // 2, seg), :])
        left = _strassen_left([[u[i * seg:(i + 1) * seg, c * KY:(c + 1) * KY].astype(F32) for c in range(2)]
                               for i in range(2)])

        def product(p):
            if p in _RIGHT_SUMS:
                return _dot(left[p], _unpack(wsum_v[_RIGHT_SUMS.index(p)]))
            c = p // 4
            return _dot(left[p], _unpack(wout_v[c * KY // 2:(c + 1) * KY // 2, c * NY:(c + 1) * NY]))

        def gate(done):
            c = _strassen_combine(lambda p: done[p] if p in done else product(p))
            return _silu_of_half(jnp.concatenate(
                [jnp.concatenate([jnp.concatenate(r, axis=1) for r in c], axis=0)
                 + _dot(u[:, 2 * KY:], _unpack(wout_v[KY:, :2 * NY])),
                 _dot(u, _unpack(wout_v[:, 2 * NY:]))], axis=1))

        mem, *first = segment(g, k, mem, side, False)
        done = {p: product(p) for p in EARLY_PRODUCTS}
        gates = None if followed else gate(done)
        mem, *second = segment(g, k + 1, mem, side, last)
        gates = gate(done) if followed else gates
        for i, (attn, late_attn) in enumerate((first, second)):
            x = x_v[_rows(4 * g + k + i, seg), :].astype(F32)
            gt = gates[i * seg:(i + 1) * seg]
            out_v[g, k + i, :early, :] = (x[:early] + attn * gt[:early]).astype(out_v.dtype)
            out_v[g, k + i, early:, NO:] = (x[early:, NO:] + late_attn * gt[early:, NO:]).astype(out_v.dtype)
            for base, t in ((GL, gt), (XL, x)):
                big_v[_rows(g, LATE, base), (k + i) * NO:(k + i + 1) * NO] = pltpu.bitcast(t[early:, :NO], U32)
        return mem

    def group(g, mem, last=False):
        previous = g - 1 if last else jnp.maximum(g - 1, 0)
        side = _SideWork([factor_slices(previous)], factor_pieces, FACTOR_FILL * 2 * heads)
        mem = segment_pair(g, 0, mem, True, side)
        mem = segment_pair(g, 2, mem, False, side, last)
        if not last:
            copy_out((g, slice(None), slice(0, early)))
        return mem

    mem = lax.fori_loop(0, n_groups - 1, group, mem_v[...].astype(F32))
    group(n_groups - 1, mem, last=True)

    ready = [[], [], [(n_groups - 1, slice(None), slice(0, early)),
                  (slice(None), slice(None), slice(early, seg), slice(NO, D))]]

    def issue_copies():
        for at in ready.pop(0):
            copy_out(at)
        ready.append([])

    def late_output(k, n, c):
        t = slice(n * LANES, (n + 1) * LANES)
        gt, x = (pltpu.bitcast(big_v[base:base + LANES, k * NO + t.start:k * NO + t.stop], F32) for base in (GL, XL))
        out_v[:, k, early:, t] = (x + c * gt).reshape(n_groups, LATE, LANES).astype(out_v.dtype)
        ready[-1].append((slice(None), k, slice(early, seg), t))

    def late_product(p, rhs):
        issue_copies()
        return _dot(pltpu.bitcast(big_v[_rows(p // 2, LANES, OF), (p % 2) * KO:(p % 2 + 1) * KO], F32), rhs)

    _strassen_squared(
        late_product, lambda k, n: _unpack(wo_v[k * KO // 2:(k + 1) * KO // 2, n * LANES:(n + 1) * LANES]), late_output,
        dtype=BF16)
    for _ in ready:
        issue_copies()
    pltpu.make_async_copy(out_v, out_hbm, sem_out).wait()


def _kernel(x_hbm, mem_hbm, wq_hbm, wk_hbm, wv_hbm, wo_hbm, wint_hbm, wsp_hbm, bsp_hbm, wout_hbm, out_hbm,
            x_v, mem_v, stage_v, wqkv_v, wo_v, wint_v, big_v, bsp_v, wout_v, wsum_v, xn_v, u_v, late_v,
            o_v, out_v, sem, sem_out, *, seg):
    _gating_branch(x_hbm, mem_hbm, wq_hbm, wk_hbm, wv_hbm, wo_hbm, wint_hbm, wsp_hbm, bsp_hbm, wout_hbm,
                   x_v, mem_v, stage_v, wqkv_v, wo_v, wint_v, big_v, bsp_v, wout_v, wsum_v, xn_v, u_v, late_v,
                   sem, seg)
    _recurrence(out_hbm, x_v, mem_v, stage_v, wqkv_v, wo_v, wout_v, wsum_v, big_v, xn_v, u_v, late_v, o_v, out_v,
                sem_out, seg)


@functools.partial(jax.jit, static_argnames=("A_seg_len",))
def pallas_recurrent_scan__memory_aug_recurrent_mem_tr__mixer_gmlp__prompt_kernel(
    A_x, A_mem0, A_Wq, A_Wk, A_Wv, A_Wo, A_seg_len, B_x, B_w_in, B_w_sp, B_b_sp, B_w_out,
):
    del B_x
    B, S, D = A_x.shape
    M = A_mem0.shape[1]
    _, H, DH = A_Wq.shape
    FH = B_w_in.shape[1] // 2
    seg = int(A_seg_len)
    assert B == 1 and DH == LANES and S == 16 * LANES and H == O_GROUPS[-1]
    assert D == 2 * KH + LANES == 2 * NY + LANES and FH == 6 * MB and 2 * KY < FH and S // seg * LATE == 4 * LANES
    big_rows = S // 2 + FH + S // 4 + FH // 2 + 13 * (FH // 4) + 4 * LANES
    groups = (S // seg // 4, 4, seg, D)
    out = pl.pallas_call(
        functools.partial(_kernel, seg=seg),
        out_shape=jax.ShapeDtypeStruct(groups, A_x.dtype),
        in_specs=[pl.BlockSpec(memory_space=pl.ANY)] * 10,
        out_specs=pl.BlockSpec(memory_space=pl.ANY),
        scratch_shapes=[
            pltpu.VMEM((S, D), BF16),
            pltpu.VMEM((M, D), BF16),
            pltpu.VMEM((H // 2, 3, 2, D // 2, DH), U32),
            pltpu.VMEM((H, D // 2, 3 * DH), U32),
            pltpu.VMEM((H * DH // 2, D), U32),
            pltpu.VMEM((2, FH // 2, D), U32),
            pltpu.VMEM((big_rows, S), U32),
            pltpu.VMEM((S // LANES, LANES), BF16),
            pltpu.VMEM((FH // 2, D), U32),
            pltpu.VMEM((5, KY // 2, NY), U32),
            pltpu.VMEM((S // 2, D), U32),
            pltpu.VMEM((S // 2, FH), U32),
            pltpu.VMEM((4, LATE, H * DH), F32),
            pltpu.VMEM((M + seg, H * DH), F32),
            pltpu.VMEM(groups, BF16),
            pltpu.SemaphoreType.DMA((24,)),
            pltpu.SemaphoreType.DMA(()),
        ],
        compiler_params=pltpu.CompilerParams(vmem_limit_bytes=120 * 1024 * 1024, disable_bounds_checks=True),
    )(
        A_x.reshape(S, D), A_mem0.reshape(M, D),
        *[w.reshape(D // 2, 2, H // 2, 2, DH) for w in (A_Wq, A_Wk, A_Wv)],
        A_Wo.reshape(H * DH, D), B_w_in.T, B_w_sp, B_b_sp.reshape(S // LANES, LANES), B_w_out,
    )
    return out.reshape(B, S, D)
```
